```python
import os as _os
_os.environ.setdefault("JAX_PLATFORMS", "cpu")
import jax
import jax.numpy as jnp

def _softmax(x, axis=-1):
    return jax.nn.softmax(x, axis=axis)
def _gelu(x):
    return jax.nn.gelu(x, approximate=True)
def _silu(x):
    return jax.nn.silu(x)
def _sigmoid(x):
    return jax.nn.sigmoid(x)
def _layernorm(x, axis=-1, eps=1e-5):
    m = jnp.mean(x, axis=axis, keepdims=True)
    v = jnp.var(x, axis=axis, keepdims=True)
    return (x - m) / jnp.sqrt(v + eps)
def _scatter_add(tgt, idx, src, axis=0):
    return tgt.at[idx].add(src)
def _segment_sum(src, seg, n):
    return jax.ops.segment_sum(src, seg, n)
class _Rng:
    def __init__(self, key):
        self._k = key
    def _next(self):
        self._k, sub = jax.random.split(self._k)
        return sub
    def normal(self, shape):
        return jax.random.normal(self._next(), shape, dtype=jnp.bfloat16)
    def randint(self, lo, hi, shape):
        return jax.random.randint(self._next(), shape, lo, hi, dtype=jnp.int32)
    def uniform(self, shape, lo=0.0, hi=1.0):
        return jax.random.uniform(self._next(), shape, jnp.bfloat16, lo, hi)
    def permutation(self, n):
        return jax.random.permutation(self._next(), n)


kernel_name = 'interleave_layers__linear_attn_block__mha_block__prompt'

def setup_inputs():
    _rng = _Rng(jax.random.key(int.from_bytes(__import__("os").urandom(4), "little")))
    _w = (lambda a: (lambda t: t.astype(jnp.bfloat16) if jnp.issubdtype(t.dtype, jnp.floating) else t)(jnp.asarray(a)))
    def _A_setup():
        B, S, D = 1, 2048, 1024
        return {
            "x": _w((lambda *s: _rng.normal(s) * 0.05)(B, S, D)),
            "wqkv": _w((lambda *s: _rng.normal(s) * 0.1)(D, 3 * D)),
            "wo": _w((lambda *s: _rng.normal(s) * 0.1)(D, D)),
        }
    _A_in = _A_setup()

    def _B_setup():
        B, S, D, H = 1, 2048, 1024, 32
        return {
            "x": _w((lambda *s: _rng.normal(s) * 0.05)(B, S, D)),
            "wqkv": _w((lambda *s: _rng.normal(s) * 0.1)(D, 3 * D)),
            "wo": _w((lambda *s: _rng.normal(s) * 0.05)(D, D)),
        }
    _B_in = _B_setup()

    return {
        "A_x": _A_in["x"],
        "A_wqkv": _A_in["wqkv"],
        "A_wo": _A_in["wo"],
        "B_x": _B_in["x"],
        "B_wqkv": _B_in["wqkv"],
        "B_wo": _B_in["wo"],
    }

def reference(A_x, A_wqkv, A_wo, B_x, B_wqkv, B_wo):
    def _A_ref(x, wqkv, wo):
        B, S, D = x.shape
        H = 32; Dh = D // H
        qkv = (lambda x, *d: x.transpose(*d))((x @ wqkv).reshape(B, S, 3, H, Dh), 2, 0, 3, 1, 4)
        q, k, v = qkv[0], qkv[1], qkv[2]
        phi = lambda t: jnp.where(t > 0, t + 1, jnp.exp(t)) + 1e-6
        pq, pk = phi(q), phi(k)
        kv = jnp.einsum("bhsd,bhse->bhde", pk, v)
        z = jnp.einsum("bhsd->bhd", pk)
        num = jnp.einsum("bhqd,bhde->bhqe", pq, kv)
        den = jnp.einsum("bhqd,bhd->bhq", pq, z)[..., None] + 1e-6
        o = num / den
        return (lambda x, *d: x.transpose(*d))(o, 0, 2, 1, 3).reshape(B, S, D) @ wo

    def _B_ref(x, wqkv, wo):
        B, S, D = x.shape
        H = 32
        Dh = D // H
        qkv = (lambda x, *d: x.transpose(*d))((x @ wqkv).reshape(B, S, 3, H, Dh), 2, 0, 3, 1, 4)
        q, k, v = qkv[0], qkv[1], qkv[2]
        scores = jnp.einsum("bhqd,bhkd->bhqk", q, k) * (Dh ** -0.5)
        p = _softmax(scores, axis=-1)
        o = jnp.einsum("bhqk,bhkd->bhqd", p, v)
        return (lambda x, *d: x.transpose(*d))(o, 0, 2, 1, 3).reshape(B, S, D) @ wo

    x = A_x
    x = x + _A_ref(_layernorm(x, axis=-1), A_wqkv, A_wo)
    x = x + _B_ref(_layernorm(x, axis=-1), B_wqkv, B_wo)
    x = x + _A_ref(_layernorm(x, axis=-1), A_wqkv, A_wo)
    x = x + _B_ref(_layernorm(x, axis=-1), B_wqkv, B_wo)
    return x
```

```python
import functools
import math

import jax
import jax.numpy as jnp
from jax import lax
import jax.experimental.pallas as pl
import jax.experimental.pallas.tpu as pltpu

S, D, H, DH = 2048, 1024, 32, 32
G = D // 128
HPG = 128 // DH
TM = 512
SUB = 256
TQ = 512
TK = 128
NQ = S // TQ
NK = S // TK
NBLK = G * NQ
WCH = 512
NWCH = 3 * D // WCH
EPS = 1e-5
QSCALE = (DH ** -0.5) * math.log2(math.e)
NT = (((1,), (1,)), ((), ()))
BF = jnp.bfloat16
F32 = jnp.float32
U32 = jnp.uint32


def _pack(v):
    return pltpu.bitcast(v.astype(BF), U32)


def _unpack(u):
    return pltpu.bitcast(u, BF)


def _ln(xt):
    mu = jnp.mean(xt, axis=-1, keepdims=True)
    xc = xt - mu
    var = jnp.mean(xc * xc, axis=-1, keepdims=True)
    return (xc * lax.rsqrt(var + EPS)).astype(BF)


def _phi(t):
    return jnp.where(t > 0, t + 1.0, jnp.exp(t)) + 1e-6


def _kernel(x_hbm, wa_hbm, woa_hbm, wb_hbm, wob_hbm, out_hbm,
            xin, x, wa, woa, wb, wob, q_s, k_s, vt_s, o_s, kv_acc, z_acc, rhs_s,
            ostage, sem_x, sem_wa, sem_w, sem_o, *bufs):
    s_bufs = bufs[:2 * HPG]
    m_bufs = bufs[2 * HPG:]

    def x_copy(t):
        return pltpu.make_async_copy(x_hbm.at[pl.ds(t * TM, TM), :], xin.at[pl.ds(t * TM, TM), :], sem_x.at[t])

    def wa_copy(c):
        return pltpu.make_async_copy(wa_hbm.at[:, pl.ds(c * WCH, WCH)], wa.at[:, pl.ds(c * WCH, WCH)], sem_wa.at[c])

    w_copies = [pltpu.make_async_copy(woa_hbm, woa, sem_w.at[0]),
                pltpu.make_async_copy(wb_hbm, wb, sem_w.at[1]),
                pltpu.make_async_copy(wob_hbm, wob, sem_w.at[2])]

    x_copy(0).start()
    for c in range(NWCH):
        wa_copy(c).start()
    for t in range(1, S // TM):
        x_copy(t).start()
    for cp in w_copies:
        cp.start()

    def a_proj(xn, r0):
        rh = pl.multiple_of(r0 // 2, SUB // 2)
        q = jnp.dot(xn, wa[:, 0:D], preferred_element_type=F32)
        pq = _pack(_phi(q))
        for g in range(G):
            q_s[g, pl.ds(rh, SUB // 2), :] = pq[:, g * 128:(g + 1) * 128]
        k = jnp.dot(xn, wa[:, D:2 * D], preferred_element_type=F32)
        pk = _phi(k)
        z_acc[...] += jnp.sum(pk.reshape(SUB // 8, 8, D), axis=0)
        pkb = pk.astype(BF)
        v = jnp.dot(xn, wa[:, 2 * D:3 * D], preferred_element_type=F32)
        vt = v.T.astype(BF)
        for g in range(G):
            kv_acc[g] += jnp.dot(vt[g * 128:(g + 1) * 128, :], pkb[:, g * 128:(g + 1) * 128],
                                 preferred_element_type=F32)

    def a_finalize():
        row = lax.broadcasted_iota(jnp.int32, (128, 128), 0) // DH
        col = lax.broadcasted_iota(jnp.int32, (128, 128), 1) // DH
        same = row == col
        z = jnp.sum(z_acc[...], axis=0, keepdims=True)
        for g in range(G):
            rhs_s[g, 0:128, :] = jnp.where(same, kv_acc[g], 0.0).astype(BF)
            zg = jnp.broadcast_to(z[:, g * 128:(g + 1) * 128], (128, 128))
            rhs_s[g, 128:256, :] = jnp.where(same, zg, 0.0).astype(BF)

    def a_out(r0):
        rh = pl.multiple_of(r0 // 2, SUB // 2)
        os = []
        for g in range(G):
            pq = _unpack(q_s[g, pl.ds(rh, SUB // 2), :])
            nd = lax.dot_general(pq, rhs_s[g], NT, preferred_element_type=F32)
            os.append((nd[:, 0:128] / (nd[:, 128:256] + 1e-6)).astype(BF))
        o = jnp.concatenate(os, axis=1)
        return jnp.dot(o, woa[...], preferred_element_type=F32)

    def b_proj(xn, r0):
        rh = pl.multiple_of(r0 // 2, SUB // 2)
        q = jnp.dot(xn, wb[:, 0:D], preferred_element_type=F32)
        qb = _pack(q * QSCALE)
        for g in range(G):
            q_s[g, pl.ds(rh, SUB // 2), :] = qb[:, g * 128:(g + 1) * 128]
        k = jnp.dot(xn, wb[:, D:2 * D], preferred_element_type=F32)
        kb = _pack(k)
        for g in range(G):
            k_s[g, pl.ds(rh, SUB // 2), :] = kb[:, g * 128:(g + 1) * 128]
        v = jnp.dot(xn, wb[:, 2 * D:3 * D], preferred_element_type=F32)
        vt = _pack(v.T)
        vt_s[:, pl.ds(r0, SUB)] = vt

    def b_out(r0):
        rh = pl.multiple_of(r0 // 2, SUB // 2)
        o = jnp.concatenate([_unpack(o_s[g, pl.ds(rh, SUB // 2), :]) for g in range(G)], axis=1)
        return jnp.dot(o, wob[...], preferred_element_type=F32)

    def zero_acc():
        kv_acc[...] = jnp.zeros_like(kv_acc)
        z_acc[...] = jnp.zeros_like(z_acc)

    lane = lax.broadcasted_iota(jnp.int32, (TQ // 2, 128), 1) // DH

    def decode(b):
        return b & (G - 1), b >> 3

    def get_qg(b):
        g, qi = decode(b)
        qoff = pl.multiple_of(qi * (TQ // 2), TQ // 2)
        return g, q_s[g, pl.ds(qoff, TQ // 2), :]

    def qk_chunk(g, qm, c, s_buf, m8):
        kc = _unpack(k_s[g, c * TK // 2:(c + 1) * TK // 2, :])
        s = lax.dot_general(kc, qm, NT, preferred_element_type=F32)
        s_buf[c * TK:(c + 1) * TK, :] = s
        mc = jnp.max(s.reshape(TK // 8, 8, TQ), axis=0)
        return mc if m8 is None else jnp.maximum(m8, mc)

    def attn_block(b, par):
        gc, qi = decode(b)
        gn, qn = get_qg(jnp.minimum(b + 1, NBLK - 1))
        outs = []
        for hh in range(HPG):
            cur = par * HPG + hh
            nxt = (1 - par) * HPG + hh
            s_cur, s_nxt = s_bufs[cur], s_bufs[nxt]
            qm = _unpack(jnp.where(lane == hh, qn, jnp.zeros_like(qn)))
            m = m_bufs[cur][...]
            voff = pl.multiple_of(gc * 64 + hh * 16, 16)
            l8 = None
            o = None
            m8 = None
            for c in range(NK):
                p = jnp.exp2(s_cur[c * TK:(c + 1) * TK, :] - m)
                lc = jnp.sum(p.reshape(TK // 8, 8, TQ), axis=0)
                l8 = lc if l8 is None else l8 + lc
                m8 = qk_chunk(gn, qm, c, s_nxt, m8)
                vc = _unpack(vt_s[pl.ds(voff, 16), c * TK:(c + 1) * TK])
                oc = jnp.dot(vc, p.astype(BF), preferred_element_type=F32)
                o = oc if o is None else o + oc
            m_bufs[nxt][...] = jnp.max(m8, axis=0, keepdims=True)
            l = jnp.sum(l8, axis=0, keepdims=True)
            outs.append(o / l)
        ot = jnp.concatenate(outs, axis=0)
        qoff = pl.multiple_of(qi * (TQ // 2), TQ // 2)
        o_s[gc, pl.ds(qoff, TQ // 2), :] = _pack(ot.T)

    def attention():
        g0, q0 = get_qg(0)
        for hh in range(HPG):
            qm = _unpack(jnp.where(lane == hh, q0, jnp.zeros_like(q0)))
            m8 = None
            for c in range(NK):
                m8 = qk_chunk(g0, qm, c, s_bufs[hh], m8)
            m_bufs[hh][...] = jnp.max(m8, axis=0, keepdims=True)

        def body(b, carry):
            for par in range(2):
                @pl.when((b & 1) == par)
                def _():
                    attn_block(b, par)
            return carry
        lax.fori_loop(0, NBLK, body, 0)

    zero_acc()
    for c in range(NWCH):
        wa_copy(c).wait()

    def p1(t, carry):
        x_copy(t).wait()
        for sb in range(TM // SUB):
            r0 = pl.multiple_of(t * TM + sb * SUB, SUB)
            xt = xin[pl.ds(r0, SUB), :].astype(F32)
            x[pl.ds(r0, SUB), :] = xt
            a_proj(_ln(xt), r0)
        return carry
    lax.fori_loop(0, S // TM, p1, 0)
    for cp in w_copies:
        cp.wait()

    def out_copy(t):
        return pltpu.make_async_copy(ostage.at[t & 1], out_hbm.at[pl.ds(t * TM, TM), :], sem_o.at[t & 1])

    def rep_body(rep, carry):
        a_finalize()

        def p2(t, c):
            xns = []
            for sb in range(TM // SUB):
                r0 = pl.multiple_of(t * TM + sb * SUB, SUB)
                xt = x[pl.ds(r0, SUB), :] + a_out(r0)
                x[pl.ds(r0, SUB), :] = xt
                xns.append(_ln(xt))
            for sb in range(TM // SUB):
                r0 = pl.multiple_of(t * TM + sb * SUB, SUB)
                b_proj(xns[sb], r0)
            return c
        lax.fori_loop(0, S // TM, p2, 0)

        attention()

        @pl.when(rep == 0)
        def _():
            zero_acc()

            def p4(t, c):
                xns = []
                for sb in range(TM // SUB):
                    r0 = pl.multiple_of(t * TM + sb * SUB, SUB)
                    xt = x[pl.ds(r0, SUB), :] + b_out(r0)
                    x[pl.ds(r0, SUB), :] = xt
                    xns.append(_ln(xt))
                for sb in range(TM // SUB):
                    r0 = pl.multiple_of(t * TM + sb * SUB, SUB)
                    a_proj(xns[sb], r0)
                return c
            lax.fori_loop(0, S // TM, p4, 0)

        @pl.when(rep == 1)
        def _():
            def p5(t, c):
                @pl.when(t >= 2)
                def _():
                    out_copy(t - 2).wait()
                for sb in range(TM // SUB):
                    r0 = pl.multiple_of(t * TM + sb * SUB, SUB)
                    xt = x[pl.ds(r0, SUB), :] + b_out(r0)
                    ostage[t & 1, sb * SUB:(sb + 1) * SUB, :] = xt.astype(BF)
                out_copy(t).start()
                return c
            lax.fori_loop(0, S // TM, p5, 0)
            out_copy(S // TM - 2).wait()
            out_copy(S // TM - 1).wait()
        return carry

    lax.fori_loop(0, 2, rep_body, 0)


@jax.jit
def pallas_interleave_layers__linear_attn_block__mha_block__prompt_kernel(A_x, A_wqkv, A_wo, B_x, B_wqkv, B_wo):
    del B_x
    scratch = [
        pltpu.VMEM((S, D), BF),
        pltpu.VMEM((S, D), F32),
        pltpu.VMEM((D, 3 * D), BF),
        pltpu.VMEM((D, D), BF),
        pltpu.VMEM((D, 3 * D), BF),
        pltpu.VMEM((D, D), BF),
        pltpu.VMEM((G, S // 2, 128), U32),
        pltpu.VMEM((G, S // 2, 128), U32),
        pltpu.VMEM((D // 2, S), U32),
        pltpu.VMEM((G, S // 2, 128), U32),
        pltpu.VMEM((G, 128, 128), F32),
        pltpu.VMEM((8, D), F32),
        pltpu.VMEM((G, 256, 128), BF),
        pltpu.VMEM((2, TM, D), BF),
        pltpu.SemaphoreType.DMA((S // TM,)),
        pltpu.SemaphoreType.DMA((NWCH,)),
        pltpu.SemaphoreType.DMA((3,)),
        pltpu.SemaphoreType.DMA((2,)),
    ] + [pltpu.VMEM((S, TQ), F32)] * (2 * HPG) + [pltpu.VMEM((1, TQ), F32)] * (2 * HPG)
    out = pl.pallas_call(
        _kernel,
        out_shape=jax.ShapeDtypeStruct((S, D), BF),
        in_specs=[pl.BlockSpec(memory_space=pl.ANY)] * 5,
        out_specs=pl.BlockSpec(memory_space=pl.ANY),
        scratch_shapes=scratch,
        compiler_params=pltpu.CompilerParams(vmem_limit_bytes=120 * 1024 * 1024),
    )(A_x.reshape(S, D), A_wqkv, A_wo, B_wqkv, B_wo)
    return out.reshape(1, S, D)
```

```python
import contextlib
import math

import jax
import jax.numpy as jnp
from jax import lax
import jax.experimental.pallas as pl
import jax.experimental.pallas.tpu as pltpu

S, D, H, DH = 2048, 1024, 32, 32
G = D // 128
HPG = 128 // DH
TM = 512
NTM = S // TM
SUB = 256
TQ = 512
TK = 128
NQ = S // TQ
NK = S // TK
NBLK = G * NQ
PRE = 128
KA = 128
LNC = 128
EPS = 1e-5
QSCALE = (DH ** -0.5) * math.log2(math.e)
BF = jnp.bfloat16
F32 = jnp.float32
U32 = jnp.uint32
SCOPES = False


def _scope(name):
    return jax.named_scope(name) if SCOPES else contextlib.nullcontext()


def _pack(v):
    return pltpu.bitcast(v.astype(BF), U32)


def _unpack(u):
    return pltpu.bitcast(u, BF)


def _dot(a, b):
    return jnp.dot(a, b, preferred_element_type=F32)


def _ln(xt):
    mu = jnp.mean(xt, axis=-1, keepdims=True)
    xc = xt - mu
    var = jnp.mean(xc * xc, axis=-1, keepdims=True)
    return (xc * lax.rsqrt(var + EPS)).astype(BF)


def _phi(t):
    return jnp.where(t > 0, t + 1.0, jnp.exp(t)) + 1e-6


def _recip(d):
    r = pl.reciprocal(d, approx=True)
    return r * (2.0 - d * r)


def _kernel(x_hbm, wa_hbm, woa_hbm, wb_hbm, wob_hbm, out_hbm,
            xin, x, xn_b, wq, wo, qt_s, k_s, vt_s, o_s, op_s, z_acc, m_s,
            s_buf, m_buf, sem_x, sem_wa, sem_w, sem_o):

    def x_copy(t):
        return pltpu.make_async_copy(x_hbm.at[pl.ds(t * TM, TM), :], xin.at[pl.ds(t * TM, TM), :], sem_x.at[t])

    c1 = 2 * D - KA
    wa_1 = pltpu.make_async_copy(wa_hbm.at[:, pl.ds(c1, D + KA)], wq.at[0, :, pl.ds(c1, D + KA)], sem_wa.at[0])
    wa_2 = pltpu.make_async_copy(wa_hbm.at[:, pl.ds(0, c1)], wq.at[0, :, pl.ds(0, c1)], sem_wa.at[1])

    w_copies = [pltpu.make_async_copy(woa_hbm, wo.at[0], sem_w.at[0]),
                pltpu.make_async_copy(wb_hbm, wq.at[1], sem_w.at[1]),
                pltpu.make_async_copy(wob_hbm, wo.at[1], sem_w.at[2])]

    def out_copy(t):
        return pltpu.make_async_copy(xin.at[pl.ds(t * TM, TM), :], out_hbm.at[pl.ds(t * TM, TM), :], sem_o.at[t])

    def ln_rows(r0, lo, hi):
        for c in range(lo, hi, LNC):
            xn_b[c // 2:(c + LNC) // 2, :] = _pack(_ln(x[pl.ds(r0 + c, LNC), :]))

    def ln0():
        ln_rows(0, 0, PRE)

    def q_phase(l):
        sel = l & 1
        is_a = sel == 0
        first = l == 0

        def k_part(t, lo, hi, xn, c0, cn):
            rh = pl.multiple_of(t * (TM // 2) + lo // 2, 64)
            k = _dot(xn, wq[sel, :, D + c0:D + c0 + cn])
            kk = jnp.where(is_a, _phi(k), k)
            z_acc[:, c0:c0 + cn] += jnp.sum(kk.reshape((hi - lo) // 8, 8, cn), axis=0)
            kb = _pack(kk)
            for g in range(cn // 128):
                k_s[c0 // 128 + g, pl.ds(rh, (hi - lo) // 2), :] = kb[:, g * 128:(g + 1) * 128]

        def body(t, carry):
            rt = pl.multiple_of(t * TM, TM)
            ln_rows(rt, PRE, TM)
            for lo, hi in ((0, PRE), (PRE, TM)):
                xn = _unpack(xn_b[lo // 2:hi // 2, :])
                v = _dot(xn, wq[sel, :, 2 * D:3 * D])
                vt_s[:, pl.ds(rt + lo, hi - lo)] = _pack(v.T)
            k_part(t, 0, TM, _unpack(xn_b[...]), D - KA, KA)

            rn = pl.multiple_of(jnp.minimum(t + 1, NTM - 1) * TM, TM)

            @pl.when(first)
            def _():
                @pl.when(t < NTM - 1)
                def _():
                    x_copy(t + 1).wait()
                    x[pl.ds(rn, TM), :] = xin[pl.ds(rn, TM), :].astype(F32)

                @pl.when(t == 0)
                def _():
                    wa_2.wait()
                    for tt in range(2, NTM):
                        x_copy(tt).start()
                    for cp in w_copies:
                        cp.start()

            xn_all = _unpack(xn_b[...])
            for sb in range(TM // SUB):
                r0 = pl.multiple_of(t * TM + sb * SUB, SUB)
                xn = xn_all[sb * SUB:(sb + 1) * SUB, :]
                q = _dot(xn, wq[sel, :, 0:D]).T
                qq = jnp.where(is_a, _phi(q), q * QSCALE)
                qt_s[:, pl.ds(r0, SUB)] = _pack(qq)
            ln_rows(rn, 0, PRE)
            for sb in range(TM // SUB):
                k_part(t, sb * SUB, (sb + 1) * SUB, xn_all[sb * SUB:(sb + 1) * SUB, :], 0, D - KA)
            return carry
        z_acc[...] = jnp.zeros_like(z_acc)
        lax.fori_loop(0, NTM, body, 0)

    def a_mix():
        row = lax.broadcasted_iota(jnp.int32, (128, 128), 0) // DH
        col = lax.broadcasted_iota(jnp.int32, (128, 128), 1) // DH
        same = row == col
        zrow = lax.broadcasted_iota(jnp.int32, (16, 128), 0)
        zcol = lax.broadcasted_iota(jnp.int32, (16, 128), 1) // DH
        zsel = zrow == zcol
        z = jnp.sum(z_acc[...], axis=0, keepdims=True)

        def kv(g):
            kvt = _dot(_unpack(vt_s[g * 64:(g + 1) * 64, :]), _unpack(k_s[g]))
            return jnp.where(same, kvt, 0.0).T.astype(BF)

        def fold(g, kvg):
            m_s[g * 64:(g + 1) * 64, :] = _pack(_dot(kvg, wo[0, g * 128:(g + 1) * 128, :]))

        def scale(g):
            zg = jnp.broadcast_to(z[:, g * 128:(g + 1) * 128], (16, 128))
            zl = jnp.where(zsel, zg, 0.0).astype(BF)
            for t in range(NTM):
                pqt = _unpack(qt_s[g * 64:(g + 1) * 64, t * TM:(t + 1) * TM])
                r = _recip(_dot(zl, pqt)[0:8, :] + 1e-6)
                pf = pqt.astype(F32)
                ot = jnp.concatenate(
                    [pf[j * DH:(j + 1) * DH, :] * r[j:j + 1, :] for j in range(HPG)], axis=0)
                o_s[g, t * TM // 2:(t + 1) * TM // 2, :] = _pack(ot.T)

        kvs = []
        for g in range(G):
            scale(g)
            kvs.append(kv(g))
            if g >= 2:
                fold(g - 2, kvs[g - 2])
        fold(G - 2, kvs[G - 2])
        fold(G - 1, kvs[G - 1])

    def a_out():
        def body(t, carry):
            ln0()
            for sb in range(TM // SUB):
                r0 = pl.multiple_of(t * TM + sb * SUB, SUB)
                rh = pl.multiple_of(t * (TM // 2) + sb * (SUB // 2), SUB // 2)
                o = jnp.concatenate([_unpack(o_s[g, pl.ds(rh, SUB // 2), :]) for g in range(G)], axis=1)
                x[pl.ds(r0, SUB), :] = x[pl.ds(r0, SUB), :] + _dot(o, _unpack(m_s[...]))
            return carry
        lax.fori_loop(0, NTM, body, 0)

    def decode(b):
        return b & (G - 1), b >> 3

    def get_qm(b, hh):
        g, qi = decode(b)
        qoff = pl.multiple_of(qi * TQ, TQ)
        if isinstance(hh, int):
            roff = pl.multiple_of(g * 64 + hh * 16, 16)
            parts = []
            if hh > 0:
                parts.append(jnp.zeros((hh * 16, TQ), U32))
            parts.append(qt_s[pl.ds(roff, 16), pl.ds(qoff, TQ)])
            if hh < HPG - 1:
                parts.append(jnp.zeros(((HPG - 1 - hh) * 16, TQ), U32))
            return _unpack(jnp.concatenate(parts, axis=0))
        roff = pl.multiple_of(g * 64, 64)
        qg = qt_s[pl.ds(roff, 64), pl.ds(qoff, TQ)]
        row = lax.broadcasted_iota(jnp.int32, (64, TQ), 0) // 16
        return _unpack(jnp.where(row == hh, qg, jnp.zeros_like(qg)))

    def qk_chunk(g, qm, c, hh, m8):
        kc = _unpack(k_s[g, c * TK // 2:(c + 1) * TK // 2, :])
        s = _dot(kc, qm)
        s_buf[hh, c * TK:(c + 1) * TK, :] = s
        mc = jnp.max(s.reshape(TK // 8, 8, TQ), axis=0)
        return mc if m8 is None else jnp.maximum(m8, mc)

    def out_proj(b, o):
        g, qi = decode(b)
        r0 = pl.multiple_of(qi * TQ, TQ)
        w0 = pl.multiple_of(g * 128, 128)
        xnew = x[pl.ds(r0, TQ), :] + _dot(o, wo[1, pl.ds(w0, 128), :])
        x[pl.ds(r0, TQ), :] = xnew
        xin[pl.ds(r0, TQ), :] = xnew.astype(BF)

    def lsum(p, l8):
        for r in range(TK // 16 - 1, -1, -1):
            pr = p[r * 16:r * 16 + 8, :] + p[r * 16 + 8:r * 16 + 16, :]
            l8 = pr if l8 is None else l8 + pr
        return l8

    def attn_block(b, last):
        gc, qi = decode(b)
        gn = (b + 1) & (G - 1)
        o_prev = _unpack(op_s[...])
        outs = []
        ms = [m_buf[hh] for hh in range(HPG)]
        for hh in range(HPG):
            if not last:
                qm = get_qm(b + 1, hh)
            voff = pl.multiple_of(gc * 64 + hh * 16, 16)
            l8 = None
            o = None
            m8 = None
            for c in range(NK):
                p = jnp.exp2(s_buf[hh, c * TK:(c + 1) * TK, :] - ms[hh])
                l8 = lsum(p, l8)
                if not last:
                    m8 = qk_chunk(gn, qm, c, hh, m8)
                elif c % 4 == 1:
                    piece = hh * 4 + c // 4
                    rr, cc = divmod(piece, 4)
                    r0 = (NQ - 1) * TQ + rr * 128
                    w0 = (G - 2) * 128
                    x[r0:r0 + 128, cc * 256:(cc + 1) * 256] += _dot(
                        o_prev[rr * 128:(rr + 1) * 128, :], wo[1, w0:w0 + 128, cc * 256:(cc + 1) * 256])
                vc = _unpack(vt_s[pl.ds(voff, 16), c * TK:(c + 1) * TK])
                oc = _dot(vc, p.astype(BF))
                o = oc if o is None else o + oc
            if not last:
                m_buf[hh] = jnp.max(m8, axis=0, keepdims=True)
            l = jnp.sum(l8, axis=0, keepdims=True)
            outs.append(o * _recip(l))
        if not last:
            out_proj(jnp.maximum(b - 1, 0), o_prev)
        ot = jnp.concatenate(outs, axis=0)
        if last:
            out_proj(b, ot.T.astype(BF))
        else:
            op_s[...] = _pack(ot.T)

    def attention(is_last_layer):
        op_s[...] = jnp.zeros_like(op_s)

        def pro(hh, carry):
            qm = get_qm(0, hh)
            m8 = None
            for c in range(NK):
                m8 = qk_chunk(0, qm, c, hh, m8)
            m_buf[hh] = jnp.max(m8, axis=0, keepdims=True)
            return carry
        with _scope('attn_pro'):
            lax.fori_loop(0, HPG, pro, 0)

        def body(b, carry):
            @pl.when(jnp.logical_and(is_last_layer, jnp.logical_and((b & (G - 1)) == 1, b > G)))
            def _():
                out_copy((b >> 3) - 1).start()
            attn_block(b, False)
            return carry
        with _scope('attn_loop'):
            lax.fori_loop(0, NBLK - 1, body, 0)
        with _scope('attn_epi'):
            ln0()
            attn_block(NBLK - 1, True)

    with _scope('start'):
        x_copy(0).start()
        wa_1.start()
        x_copy(0).wait()
        x[0:TM, :] = xin[0:TM, :].astype(F32)
        ln0()
        wa_1.wait()
        x_copy(1).start()
        wa_2.start()

    def layer(l, carry):
        sel = l & 1
        with _scope('q_phase'):
            q_phase(l)

        @pl.when(l == 0)
        def _():
            for cp in w_copies:
                cp.wait()

        @pl.when(sel == 0)
        def _():
            with _scope('a_mix'):
                a_mix()
            with _scope('a_out'):
                a_out()

        @pl.when(sel == 1)
        def _():
            attention(l == 3)
        return carry

    lax.fori_loop(0, 4, layer, 0)
    out_copy(NTM - 1).start()
    for t in range(NTM):
        out_copy(t).wait()


@jax.jit
def pallas_interleave_layers__linear_attn_block__mha_block__prompt_kernel(A_x, A_wqkv, A_wo, B_x, B_wqkv, B_wo):
    del B_x
    scratch = [
        pltpu.VMEM((S, D), BF),
        pltpu.VMEM((S, D), F32),
        pltpu.VMEM((TM // 2, D), U32),
        pltpu.VMEM((2, D, 3 * D), BF),
        pltpu.VMEM((2, D, D), BF),
        pltpu.VMEM((D // 2, S), U32),
        pltpu.VMEM((G, S // 2, 128), U32),
        pltpu.VMEM((D // 2, S), U32),
        pltpu.VMEM((G, S // 2, 128), U32),
        pltpu.VMEM((TQ // 2, 128), U32),
        pltpu.VMEM((8, D), F32),
        pltpu.VMEM((D // 2, D), U32),
        pltpu.VMEM((HPG, S, TQ), F32),
        pltpu.VMEM((HPG, 1, TQ), F32),
        pltpu.SemaphoreType.DMA((NTM,)),
        pltpu.SemaphoreType.DMA((2,)),
        pltpu.SemaphoreType.DMA((3,)),
        pltpu.SemaphoreType.DMA((NTM,)),
    ]
    out = pl.pallas_call(
        _kernel,
        out_shape=jax.ShapeDtypeStruct((S, D), BF),
        in_specs=[pl.BlockSpec(memory_space=pl.ANY)] * 5,
        out_specs=pl.BlockSpec(memory_space=pl.ANY),
        scratch_shapes=scratch,
        compiler_params=pltpu.CompilerParams(vmem_limit_bytes=120 * 1024 * 1024),
    )(A_x.reshape(S, D), A_wqkv, A_wo, B_wqkv, B_wo)
    return out.reshape(1, S, D)
```

```python
import contextlib
import math

import jax
import jax.numpy as jnp
from jax import lax
import jax.experimental.pallas as pl
import jax.experimental.pallas.tpu as pltpu

S, D, H, DH = 2048, 1024, 32, 32
G = D // 128
HPG = 128 // DH
TM = 512
NTM = S // TM
SUB = 256
TQ = 512
TK = 128
NQ = S // TQ
NK = S // TK
NBLK = G * NQ
PRE = 128
KA = 128
LNC = 128
EPS = 1e-5
WPAD = 256
QSCALE = (DH ** -0.5) * math.log2(math.e)
BF = jnp.bfloat16
F32 = jnp.float32
U32 = jnp.uint32
SCOPES = False


def _scope(name):
    return jax.named_scope(name) if SCOPES else contextlib.nullcontext()


def _pack(v):
    return pltpu.bitcast(v.astype(BF), U32)


def _unpack(u):
    return pltpu.bitcast(u, BF)


def _dot(a, b):
    return jnp.dot(a, b, preferred_element_type=F32)


def _ln(xt):
    mu = jnp.mean(xt, axis=-1, keepdims=True)
    xc = xt - mu
    var = jnp.mean(xc * xc, axis=-1, keepdims=True)
    return (xc * lax.rsqrt(var + EPS)).astype(BF)


def _phi(t):
    return jnp.where(t > 0, t + 1.0, jnp.exp(t)) + 1e-6


def _recip(d):
    r = pl.reciprocal(d, approx=True)
    return r * (2.0 - d * r)


def _kernel(x_hbm, wa_hbm, woa_hbm, wb_hbm, wob_hbm, out_hbm,
            xin, x, xn_b, wq, wo, qt_s, k_s, vt_s, o_s, op_s, z_acc, m_s, zero_s,
            s_buf, m_buf, sem_x, sem_wa, sem_w, sem_o):

    def x_copy(t):
        return pltpu.make_async_copy(x_hbm.at[pl.ds(t * TM, TM), :], xin.at[pl.ds(t * TM, TM), :], sem_x.at[t])

    c1 = 2 * D - KA
    wa_1 = pltpu.make_async_copy(wa_hbm.at[:, pl.ds(c1, D + KA)], wq.at[0, :, pl.ds(c1, D + KA)], sem_wa.at[0])
    wa_2 = pltpu.make_async_copy(wa_hbm.at[:, pl.ds(0, c1)], wq.at[0, :, pl.ds(0, c1)], sem_wa.at[1])

    w_copies = [pltpu.make_async_copy(woa_hbm, wo.at[0, :, pl.ds(0, D)], sem_w.at[0]),
                pltpu.make_async_copy(wb_hbm, wq.at[1, :, pl.ds(0, 3 * D)], sem_w.at[1]),
                pltpu.make_async_copy(wob_hbm, wo.at[1, :, pl.ds(0, D)], sem_w.at[2])]

    def out_copy(t):
        return pltpu.make_async_copy(xin.at[pl.ds(t * TM, TM), :], out_hbm.at[pl.ds(t * TM, TM), :], sem_o.at[t])

    def out_copy_last(j):
        r0 = (NTM - 1) * TM + j * 128
        return pltpu.make_async_copy(xin.at[pl.ds(r0, 128), :], out_hbm.at[pl.ds(r0, 128), :],
                                     sem_o.at[NTM - 1 + j])

    def ln_rows(r0, lo, hi):
        for c in range(lo, hi, LNC):
            xn_b[c // 2:(c + LNC) // 2, :] = _pack(_ln(x[pl.ds(r0 + c, LNC), :]))

    def ln0():
        ln_rows(0, 0, PRE)

    def q_phase(l):
        sel = l & 1
        is_a = sel == 0
        first = l == 0

        def k_part(t, lo, hi, xn, c0, cn):
            rh = pl.multiple_of(t * (TM // 2) + lo // 2, 64)
            k = _dot(xn, wq[sel, :, D + c0:D + c0 + cn])
            kk = jnp.where(is_a, _phi(k), k)
            z_acc[:, c0:c0 + cn] += jnp.sum(kk.reshape((hi - lo) // 8, 8, cn), axis=0)
            kb = _pack(kk)
            for g in range(cn // 128):
                k_s[c0 // 128 + g, pl.ds(rh, (hi - lo) // 2), :] = kb[:, g * 128:(g + 1) * 128]

        def body(t, carry):
            rt = pl.multiple_of(t * TM, TM)
            ln_rows(rt, PRE, TM)
            for lo, hi in ((0, PRE), (PRE, TM)):
                xn = _unpack(xn_b[lo // 2:hi // 2, :])
                v = _dot(xn, wq[sel, :, 2 * D:3 * D])
                vt_s[:, pl.ds(rt + lo, hi - lo)] = _pack(v.T)
            k_part(t, 0, TM, _unpack(xn_b[...]), D - KA, KA)

            rn = pl.multiple_of(jnp.minimum(t + 1, NTM - 1) * TM, TM)

            @pl.when(first)
            def _():
                @pl.when(t < NTM - 1)
                def _():
                    x_copy(t + 1).wait()
                    x[pl.ds(rn, TM), :] = xin[pl.ds(rn, TM), :].astype(F32)

                @pl.when(t == 0)
                def _():
                    wa_2.wait()
                    for tt in range(2, NTM):
                        x_copy(tt).start()
                    for cp in w_copies:
                        cp.start()

            xn_all = _unpack(xn_b[...])
            for sb in range(TM // SUB):
                r0 = pl.multiple_of(t * TM + sb * SUB, SUB)
                xn = xn_all[sb * SUB:(sb + 1) * SUB, :]
                q = _dot(xn, wq[sel, :, 0:D]).T
                qq = jnp.where(is_a, _phi(q), q * QSCALE)
                qt_s[:, pl.ds(r0, SUB)] = _pack(qq)
            ln_rows(rn, 0, PRE)
            for sb in range(TM // SUB):
                k_part(t, sb * SUB, (sb + 1) * SUB, xn_all[sb * SUB:(sb + 1) * SUB, :], 0, D - KA)
            return carry
        z_acc[...] = jnp.zeros_like(z_acc)
        lax.fori_loop(0, NTM, body, 0)

    def a_mix():
        row = lax.broadcasted_iota(jnp.int32, (128, 128), 0) // DH
        col = lax.broadcasted_iota(jnp.int32, (128, 128), 1) // DH
        same = row == col
        zrow = lax.broadcasted_iota(jnp.int32, (16, 128), 0)
        zcol = lax.broadcasted_iota(jnp.int32, (16, 128), 1) // DH
        zsel = zrow == zcol
        z = jnp.sum(z_acc[...], axis=0, keepdims=True)

        def fold(g, kvg):
            m_s[g * 64:(g + 1) * 64, :] = _pack(_dot(kvg, wo[0, g * 128:(g + 1) * 128, 0:D]))

        def group(g):
            zg = jnp.broadcast_to(z[:, g * 128:(g + 1) * 128], (16, 128))
            zl = jnp.where(zsel, zg, 0.0).astype(BF)
            kvt = None
            for t in range(NTM):
                pqt = _unpack(qt_s[g * 64:(g + 1) * 64, t * TM:(t + 1) * TM])
                r = _recip(_dot(zl, pqt)[0:8, :] + 1e-6)
                pf = pqt.astype(F32)
                ot = jnp.concatenate(
                    [pf[j * DH:(j + 1) * DH, :] * r[j:j + 1, :] for j in range(HPG)], axis=0)
                o_s[g, t * TM // 2:(t + 1) * TM // 2, :] = _pack(ot.T)
                part = _dot(_unpack(vt_s[g * 64:(g + 1) * 64, t * TM:(t + 1) * TM]),
                            _unpack(k_s[g, t * TM // 2:(t + 1) * TM // 2, :]))
                kvt = part if kvt is None else kvt + part
            return jnp.where(same, kvt, 0.0).T.astype(BF)

        kvs = []
        for g in range(G):
            kvs.append(group(g))
            if g >= 2:
                fold(g - 2, kvs[g - 2])
        fold(G - 2, kvs[G - 2])
        fold(G - 1, kvs[G - 1])

    def a_out():
        def body(t, carry):
            ln0()
            for sb in range(TM // SUB):
                r0 = pl.multiple_of(t * TM + sb * SUB, SUB)
                rh = pl.multiple_of(t * (TM // 2) + sb * (SUB // 2), SUB // 2)
                o = jnp.concatenate([_unpack(o_s[g, pl.ds(rh, SUB // 2), :]) for g in range(G)], axis=1)
                x[pl.ds(r0, SUB), :] = x[pl.ds(r0, SUB), :] + _dot(o, _unpack(m_s[...]))
            return carry
        lax.fori_loop(0, NTM, body, 0)

    def decode(b):
        return b & (G - 1), b >> 3

    def get_qm(b, hh):
        g, qi = decode(b)
        qoff = pl.multiple_of(qi * TQ, TQ)
        if isinstance(hh, int):
            roff = pl.multiple_of(g * 64 + hh * 16, 16)
            parts = []
            if hh > 0:
                parts.append(jnp.zeros((hh * 16, TQ), U32))
            parts.append(qt_s[pl.ds(roff, 16), pl.ds(qoff, TQ)])
            if hh < HPG - 1:
                parts.append(jnp.zeros(((HPG - 1 - hh) * 16, TQ), U32))
            return _unpack(jnp.concatenate(parts, axis=0))
        roff = pl.multiple_of(g * 64, 64)
        qg = qt_s[pl.ds(roff, 64), pl.ds(qoff, TQ)]
        row = lax.broadcasted_iota(jnp.int32, (64, TQ), 0) // 16
        return _unpack(jnp.where(row == hh, qg, jnp.zeros_like(qg)))

    def qk_chunk(g, qm, c, hh, m8):
        kc = _unpack(k_s[g, c * TK // 2:(c + 1) * TK // 2, :])
        s = _dot(kc, qm)
        s_buf[hh, c * TK:(c + 1) * TK, :] = s
        mc = jnp.max(s.reshape(TK // 8, 8, TQ), axis=0)
        return mc if m8 is None else jnp.maximum(m8, mc)

    def out_proj(b, o):
        g, qi = decode(b)
        r0 = pl.multiple_of(qi * TQ, TQ)
        w0 = pl.multiple_of(g * 128, 128)
        xnew = x[pl.ds(r0, TQ), :] + _dot(o, wo[1, pl.ds(w0, 128), 0:D])
        x[pl.ds(r0, TQ), :] = xnew
        xin[pl.ds(r0, TQ), :] = xnew.astype(BF)

    def lsum(p, l8):
        for r in range(TK // 16 - 1, -1, -1):
            pr = p[r * 16:r * 16 + 8, :] + p[r * 16 + 8:r * 16 + 16, :]
            l8 = pr if l8 is None else l8 + pr
        return l8

    def attn_block(b):
        gc, qi = decode(b)
        gn = (b + 1) & (G - 1)
        o_prev = _unpack(op_s[...])
        outs = []
        ms = [m_buf[hh] for hh in range(HPG)]
        for hh in range(HPG):
            qm = get_qm(b + 1, hh)
            voff = pl.multiple_of(gc * 64 + hh * 16, 16)
            l8 = None
            o = zero_s[...]
            m8 = None
            for c in range(NK):
                p = jnp.exp2(s_buf[hh, c * TK:(c + 1) * TK, :] - ms[hh])
                l8 = lsum(p, l8)
                m8 = qk_chunk(gn, qm, c, hh, m8)
                vc = _unpack(vt_s[pl.ds(voff, 16), c * TK:(c + 1) * TK])
                o = o + _dot(vc, p.astype(BF))
            m_buf[hh] = jnp.max(m8, axis=0, keepdims=True)
            l = jnp.sum(l8, axis=0, keepdims=True)
            outs.append(o * _recip(l))
        out_proj(jnp.maximum(b - 1, 0), o_prev)
        ot = jnp.concatenate(outs, axis=0)
        op_s[...] = _pack(ot.T)

    def attn_last(is_last_layer):
        EQ = 256
        EK = 256
        rbase = (NQ - 1) * TQ

        def proj_piece(o, g, r, cc, final):
            r0 = rbase + r
            cols = slice(cc * 256, (cc + 1) * 256)
            xnew = x[r0:r0 + 128, cols] + _dot(o, wo[1, g * 128:(g + 1) * 128, cols])
            x[r0:r0 + 128, cols] = xnew
            if final:
                xin[r0:r0 + 128, cols] = xnew.astype(BF)
                if cc == 3:
                    @pl.when(is_last_layer)
                    def _():
                        out_copy_last(r // 128).start()

        o_prev = _unpack(op_s[...])
        queue = [(o_prev[r:r + 128, :], G - 2, r, cc, False) for r in range(0, TQ, 128) for cc in range(4)]
        for j in range(TQ // EQ):
            cols = slice(j * EQ, (j + 1) * EQ)
            outs = []
            step = 0
            for hh in range(HPG):
                m = m_buf[hh, :, cols]
                voff = (G - 1) * 64 + hh * 16
                l8 = None
                o = zero_s[:, 0:EQ]
                for c in range(S // EK):
                    p = jnp.exp2(s_buf[hh, c * EK:(c + 1) * EK, cols] - m)
                    for u in range(EK // TK):
                        l8 = lsum(p[u * TK:(u + 1) * TK, :], l8)
                    vc = _unpack(vt_s[voff:voff + 16, c * EK:(c + 1) * EK])
                    o = o + _dot(vc, p.astype(BF))
                    step += 1
                    if queue and step % 8 in (1, 4, 6):
                        proj_piece(*queue.pop(0))
                l = jnp.sum(l8, axis=0, keepdims=True)
                outs.append(o * _recip(l))
            oj = jnp.concatenate(outs, axis=0).T.astype(BF)
            queue += [(oj[r:r + 128, :], G - 1, j * EQ + r, cc, True) for r in range(0, EQ, 128) for cc in range(4)]
        while queue:
            proj_piece(*queue.pop(0))

    def attention(is_last_layer):
        op_s[...] = jnp.zeros_like(op_s)

        def pro(i, carry):
            for u in range(2):
                hh = 2 * i + u
                qm = get_qm(0, hh)
                m8 = None
                for c in range(NK):
                    m8 = qk_chunk(0, qm, c, hh, m8)
                m_buf[hh] = jnp.max(m8, axis=0, keepdims=True)
            return carry
        with _scope('attn_pro'):
            lax.fori_loop(0, HPG // 2, pro, 0)

        def body(b, carry):
            @pl.when(jnp.logical_and(is_last_layer, jnp.logical_and((b & (G - 1)) == 1, b > G)))
            def _():
                out_copy((b >> 3) - 1).start()
            attn_block(b)
            return carry
        with _scope('attn_loop'):
            lax.fori_loop(0, NBLK - 1, body, 0)
        with _scope('attn_epi'):
            ln0()
            attn_last(is_last_layer)

    with _scope('start'):
        x_copy(0).start()
        wa_1.start()
        zero_s[...] = jnp.zeros_like(zero_s)
        x_copy(0).wait()
        x[0:TM, :] = xin[0:TM, :].astype(F32)
        ln0()
        wa_1.wait()
        x_copy(1).start()
        wa_2.start()

    def layer(l, carry):
        sel = l & 1
        with _scope('q_phase'):
            q_phase(l)

        @pl.when(l == 0)
        def _():
            for cp in w_copies:
                cp.wait()

        @pl.when(sel == 0)
        def _():
            with _scope('a_mix'):
                a_mix()
            with _scope('a_out'):
                a_out()

        @pl.when(sel == 1)
        def _():
            attention(l == 3)
        return carry

    lax.fori_loop(0, 4, layer, 0)
    for t in range(NTM - 1):
        out_copy(t).wait()
    for j in range(TM // 128):
        out_copy_last(j).wait()


@jax.jit
def pallas_interleave_layers__linear_attn_block__mha_block__prompt_kernel(A_x, A_wqkv, A_wo, B_x, B_wqkv, B_wo):
    del B_x
    scratch = [
        pltpu.VMEM((S, D), BF),
        pltpu.VMEM((S, D), F32),
        pltpu.VMEM((TM // 2, D), U32),
        pltpu.VMEM((2, D, 3 * D + WPAD), BF),
        pltpu.VMEM((2, D, D + WPAD), BF),
        pltpu.VMEM((D // 2, S), U32),
        pltpu.VMEM((G, S // 2, 128), U32),
        pltpu.VMEM((D // 2, S), U32),
        pltpu.VMEM((G, S // 2, 128), U32),
        pltpu.VMEM((TQ // 2, 128), U32),
        pltpu.VMEM((8, D), F32),
        pltpu.VMEM((D // 2, D), U32),
        pltpu.VMEM((DH, TQ), F32),
        pltpu.VMEM((HPG, S, TQ), F32),
        pltpu.VMEM((HPG, 1, TQ), F32),
        pltpu.SemaphoreType.DMA((NTM,)),
        pltpu.SemaphoreType.DMA((2,)),
        pltpu.SemaphoreType.DMA((3,)),
        pltpu.SemaphoreType.DMA((NTM - 1 + TM // 128,)),
    ]
    out = pl.pallas_call(
        _kernel,
        out_shape=jax.ShapeDtypeStruct((S, D), BF),
        in_specs=[pl.BlockSpec(memory_space=pl.ANY)] * 5,
        out_specs=pl.BlockSpec(memory_space=pl.ANY),
        scratch_shapes=scratch,
        compiler_params=pltpu.CompilerParams(vmem_limit_bytes=120 * 1024 * 1024),
    )(A_x.reshape(S, D), A_wqkv, A_wo, B_wqkv, B_wo)
    return out.reshape(1, S, D)
```

```python
import contextlib
import math

import jax
import jax.numpy as jnp
from jax import lax
import jax.experimental.pallas as pl
import jax.experimental.pallas.tpu as pltpu

S, D, H, DH = 2048, 1024, 32, 32
G = D // 128
HPG = 128 // DH
TM = 512
NTM = S // TM
SUB = 256
TQ = 512
TK = 128
NQ = S // TQ
NK = S // TK
NBLK = G * NQ
PRE = 128
KA = 128
LNC = 32
EPS = 1e-5
WPAD = 256
QSCALE = (DH ** -0.5) * math.log2(math.e)
BF = jnp.bfloat16
F32 = jnp.float32
U32 = jnp.uint32
SCOPES = False


def _scope(name):
    return jax.named_scope(name) if SCOPES else contextlib.nullcontext()


def _pack(v):
    return pltpu.bitcast(v.astype(BF), U32)


def _unpack(u):
    return pltpu.bitcast(u, BF)


def _dot(a, b):
    return jnp.dot(a, b, preferred_element_type=F32)


def _ln(xt):
    mu = jnp.mean(xt, axis=-1, keepdims=True)
    xc = xt - mu
    var = jnp.mean(xc * xc, axis=-1, keepdims=True)
    return (xc * lax.rsqrt(var + EPS)).astype(BF)


def _zero_of(v):
    return pltpu.bitcast(pltpu.bitcast(v, U32) & jnp.uint32(0x80000000), F32)


def _phi(t):
    return jnp.where(t > 0, t + 1.0, jnp.exp(t)) + 1e-6


def _recip(d):
    r = pl.reciprocal(d, approx=True)
    return r * (2.0 - d * r)


def _kernel(x_hbm, wa_hbm, woa_hbm, wb_hbm, wob_hbm, out_hbm,
            xin, x, xn_b, xn_0, wq, wo, t_s, k_s, o_s, op_s, z_acc, m_s, zero_s,
            s_buf, m_buf, sem_x0, sem_wa, sem_w, sem_o):

    XC = S // G

    def x_copy(i):
        r0 = pl.multiple_of(i * XC, XC)
        return pltpu.make_async_copy(x_hbm.at[pl.ds(r0, XC), :], xin.at[pl.ds(r0, XC), :], sem_wa.at[i & 1])

    x0_rows = [(i * 32, 32) for i in range(8)] + [(256 + i * 64, 64) for i in range(4)]
    x0_copies = [pltpu.make_async_copy(x_hbm.at[pl.ds(r, n), :], xin.at[pl.ds(r, n), :], sem_x0.at[i // 8])
                 for i, (r, n) in enumerate(x0_rows)]

    def t_col(j):
        return (1 - (j >> 2)) * (2 * D) + (j & 3) * 256

    def wa_copies(j):
        ct = pl.multiple_of(t_col(j), 256) if not isinstance(j, int) else t_col(j)
        ck = pl.multiple_of(D + j * 128, 128) if not isinstance(j, int) else D + j * 128
        return (pltpu.make_async_copy(wa_hbm.at[:, pl.ds(ct, 256)], wq.at[0, :, pl.ds(ct, 256)], sem_wa.at[j & 1]),
                pltpu.make_async_copy(wa_hbm.at[:, pl.ds(ck, 128)], wq.at[0, :, pl.ds(ck, 128)], sem_wa.at[j & 1]))

    w_copies = [pltpu.make_async_copy(woa_hbm, wo.at[0, :, pl.ds(0, D)], sem_w.at[0]),
                pltpu.make_async_copy(wb_hbm, wq.at[1, :, pl.ds(0, 3 * D)], sem_w.at[0]),
                pltpu.make_async_copy(wob_hbm, wo.at[1, :, pl.ds(0, D)], sem_w.at[0])]

    def out_copy(t):
        return pltpu.make_async_copy(xin.at[pl.ds(t * TM, TM), :], out_hbm.at[pl.ds(t * TM, TM), :], sem_o.at[0])

    def out_copy_last(j):
        r0 = (NTM - 1) * TM + j * 128
        return pltpu.make_async_copy(xin.at[pl.ds(r0, 128), :], out_hbm.at[pl.ds(r0, 128), :],
                                     sem_o.at[0])

    def ln_rows(r0, lo, hi, dep=None):
        paced = dep is not None
        for c in range(lo, hi, LNC):
            xt = x[pl.ds(r0 + c, LNC), :]
            acc = xt[:, 0:128] + dep if paced else xt[:, 0:128]
            for j in range(1, D // 128):
                acc = acc + xt[:, j * 128:(j + 1) * 128]
            mu = jnp.sum(acc, axis=-1, keepdims=True) * (1.0 / D)
            xc = xt - mu
            var = jnp.mean(xc * xc, axis=-1, keepdims=True)
            r = lax.rsqrt(var + EPS)
            xn_b[c // 2:(c + LNC) // 2, :] = _pack(xc * r)
            dep = _zero_of(r)
        return dep

    def ln0():
        ln_rows(0, 0, PRE)

    def q_phase(l):
        sel = l & 1
        is_a = sel == 0
        first = l == 0

        def k_part(t, lo, hi, xn, c0, cn):
            rh = pl.multiple_of(t * (TM // 2) + lo // 2, 64)
            k = _dot(xn, wq[sel, :, D + c0:D + c0 + cn])
            kk = jnp.where(is_a, _phi(k), k)
            z_acc[:, c0:c0 + cn] += jnp.sum(kk.reshape((hi - lo) // 8, 8, cn), axis=0)
            kb = _pack(kk)
            for g in range(cn // 128):
                k_s[c0 // 128 + g, pl.ds(rh, (hi - lo) // 2), :] = kb[:, g * 128:(g + 1) * 128]

        def body(t, carry):
            rt = pl.multiple_of(t * TM, TM)
            rn = pl.multiple_of(jnp.minimum(t + 1, NTM - 1) * TM, TM)
            ln_rows(rt, PRE, TM)
            xn_all = _unpack(xn_b[...])
            for lo, hi in ((0, PRE), (PRE, TM)):
                v = _dot(xn_all[lo:hi, :], wq[sel, :, 2 * D:3 * D])
                t_s[1, :, pl.ds(rt + lo, hi - lo)] = _pack(v.T)
            for sb in range(TM // SUB):
                r0 = pl.multiple_of(t * TM + sb * SUB, SUB)
                xn = xn_all[sb * SUB:(sb + 1) * SUB, :]
                q = _dot(xn, wq[sel, :, 0:D]).T
                qq = jnp.where(is_a, _phi(q), q * QSCALE)
                t_s[0, :, pl.ds(r0, SUB)] = _pack(qq)
                if sb == 0:
                    dep = _zero_of(qq[0:LNC, 0:128])
            ln_rows(rn, 0, PRE, dep)
            for sb in range(TM // SUB):
                k_part(t, sb * SUB, (sb + 1) * SUB, xn_all[sb * SUB:(sb + 1) * SUB, :], 0, D)
            return carry

        @pl.when(l > 0)
        def _():
            z_acc[...] = jnp.zeros_like(z_acc)
        lax.fori_loop(jnp.where(first, 1, 0), NTM, body, 0)

    def startup():
        for cp in x0_copies:
            cp.start()
        for cp in wa_copies(0):
            cp.start()
        zero_s[...] = jnp.zeros_like(zero_s)
        for cp in x0_copies[:8]:
            cp.wait()
        xn_0[0:128, :] = _pack(_ln(xin[0:256, :].astype(F32)))
        for cp in x0_copies[8:]:
            cp.wait()
        xn_0[128:256, :] = _pack(_ln(xin[256:512, :].astype(F32)))
        for cp in wa_copies(1):
            cp.start()
        for cp in wa_copies(0):
            cp.wait()

        def body(j, carry):
            xn = _unpack(xn_0[...])
            ct = pl.multiple_of(t_col(j), 256)
            ck = pl.multiple_of(j * 128, 128)
            rc = pl.multiple_of(j * XC, XC)
            xf = xin[pl.ds(rc, XC), :].astype(F32)
            x[pl.ds(rc, XC), :] = xf
            u = pltpu.bitcast(xf, U32)
            u = u[:, 0:512] | u[:, 512:1024]
            u = jnp.concatenate([u[:, 0:256], u[:, 256:512]], axis=0) & jnp.uint32(0x80000000)
            y = (_dot(xn, wq[0, :, pl.ds(ct, 256)]) + pltpu.bitcast(u, F32)).T
            y = jnp.where(j >= 4, _phi(y), y)
            tr = pl.multiple_of((j & 3) * 128, 128)
            t_s[1 - (j >> 2), pl.ds(tr, 128), 0:TM] = _pack(y)
            kk = _phi(_dot(xn, wq[0, :, pl.ds(D + ck, 128)]))
            z_acc[:, pl.ds(ck, 128)] = jnp.sum(kk.reshape(TM // 8, 8, 128), axis=0)
            k_s[j, 0:TM // 2, :] = _pack(kk)

            @pl.when(j + 2 < G)
            def _():
                x_copy(j + 2).start()
                for cp in wa_copies(j + 2):
                    cp.start()

            @pl.when(j == G - 2)
            def _():
                for cp in w_copies:
                    cp.start()

            @pl.when(j + 1 < G)
            def _():
                for cp in wa_copies(j + 1):
                    cp.wait()

                @pl.when(j > 0)
                def _():
                    x_copy(j + 1).wait()
            return carry
        lax.fori_loop(0, G, body, 0)
        ln_rows(TM, 0, PRE)

    def a_mix():
        row = lax.broadcasted_iota(jnp.int32, (128, 128), 0) // DH
        col = lax.broadcasted_iota(jnp.int32, (128, 128), 1) // DH
        same = row == col
        zrow = lax.broadcasted_iota(jnp.int32, (16, 128), 0)
        zcol = lax.broadcasted_iota(jnp.int32, (16, 128), 1) // DH
        zsel = zrow == zcol
        z = jnp.sum(z_acc[...], axis=0, keepdims=True)

        def fold(g, kvg):
            m_s[g * 64:(g + 1) * 64, :] = _pack(_dot(kvg, wo[0, g * 128:(g + 1) * 128, 0:D]))

        def group(g):
            zg = jnp.broadcast_to(z[:, g * 128:(g + 1) * 128], (16, 128))
            zl = jnp.where(zsel, zg, 0.0).astype(BF)
            kvt = None
            for t in range(NTM):
                pqt = _unpack(t_s[0, g * 64:(g + 1) * 64, t * TM:(t + 1) * TM])
                r = _recip(_dot(zl, pqt)[0:8, :] + 1e-6)
                pf = pqt.astype(F32)
                ot = jnp.concatenate(
                    [pf[j * DH:(j + 1) * DH, :] * r[j:j + 1, :] for j in range(HPG)], axis=0)
                o_s[g, t * TM // 2:(t + 1) * TM // 2, :] = _pack(ot.T)
                part = _dot(_unpack(t_s[1, g * 64:(g + 1) * 64, t * TM:(t + 1) * TM]),
                            _unpack(k_s[g, t * TM // 2:(t + 1) * TM // 2, :]))
                kvt = part if kvt is None else kvt + part
            return jnp.where(same, kvt, 0.0).T.astype(BF)

        kvs = []
        for g in range(G):
            kvs.append(group(g))
            if g >= 2:
                fold(g - 2, kvs[g - 2])
        fold(G - 2, kvs[G - 2])
        fold(G - 1, kvs[G - 1])

    def a_out():
        def body(t, carry):
            ln0()
            for sb in range(TM // SUB):
                r0 = pl.multiple_of(t * TM + sb * SUB, SUB)
                rh = pl.multiple_of(t * (TM // 2) + sb * (SUB // 2), SUB // 2)
                o = jnp.concatenate([_unpack(o_s[g, pl.ds(rh, SUB // 2), :]) for g in range(G)], axis=1)
                x[pl.ds(r0, SUB), :] = x[pl.ds(r0, SUB), :] + _dot(o, _unpack(m_s[...]))
            return carry
        lax.fori_loop(0, NTM, body, 0)

    def decode(b):
        return b & (G - 1), b >> 3

    def get_qm(b, hh):
        g, qi = decode(b)
        qoff = pl.multiple_of(qi * TQ, TQ)
        if isinstance(hh, int):
            roff = pl.multiple_of(g * 64 + hh * 16, 16)
            parts = []
            if hh > 0:
                parts.append(jnp.zeros((hh * 16, TQ), U32))
            parts.append(t_s[0, pl.ds(roff, 16), pl.ds(qoff, TQ)])
            if hh < HPG - 1:
                parts.append(jnp.zeros(((HPG - 1 - hh) * 16, TQ), U32))
            return _unpack(jnp.concatenate(parts, axis=0))
        roff = pl.multiple_of(g * 64, 64)
        qg = t_s[0, pl.ds(roff, 64), pl.ds(qoff, TQ)]
        row = lax.broadcasted_iota(jnp.int32, (64, TQ), 0) // 16
        return _unpack(jnp.where(row == hh, qg, jnp.zeros_like(qg)))

    def qk_chunk(g, qm, c, hh, m8):
        kc = _unpack(k_s[g, c * TK // 2:(c + 1) * TK // 2, :])
        s = _dot(kc, qm)
        s_buf[hh, c * TK:(c + 1) * TK, :] = s
        mc = jnp.max(s.reshape(TK // 8, 8, TQ), axis=0)
        return mc if m8 is None else jnp.maximum(m8, mc)

    def out_proj(b, o):
        g, qi = decode(b)
        r0 = pl.multiple_of(qi * TQ, TQ)
        w0 = pl.multiple_of(g * 128, 128)
        xnew = x[pl.ds(r0, TQ), :] + _dot(o, wo[1, pl.ds(w0, 128), 0:D])
        x[pl.ds(r0, TQ), :] = xnew
        xin[pl.ds(r0, TQ), :] = xnew.astype(BF)

    def lsum(p, l8):
        for r in range(TK // 16 - 1, -1, -1):
            pr = p[r * 16:r * 16 + 8, :] + p[r * 16 + 8:r * 16 + 16, :]
            l8 = pr if l8 is None else l8 + pr
        return l8

    def attn_block(b):
        gc, qi = decode(b)
        gn = (b + 1) & (G - 1)
        o_prev = _unpack(op_s[...])
        outs = []
        ms = [m_buf[hh] for hh in range(HPG)]
        for hh in range(HPG):
            qm = get_qm(b + 1, hh)
            voff = pl.multiple_of(gc * 64 + hh * 16, 16)
            l8 = None
            o = zero_s[...]
            m8 = None
            for c in range(NK):
                p = jnp.exp2(s_buf[hh, c * TK:(c + 1) * TK, :] - ms[hh])
                l8 = lsum(p, l8)
                m8 = qk_chunk(gn, qm, c, hh, m8)
                vc = _unpack(t_s[1, pl.ds(voff, 16), c * TK:(c + 1) * TK])
                o = o + _dot(vc, p.astype(BF))
            m_buf[hh] = jnp.max(m8, axis=0, keepdims=True)
            l = jnp.sum(l8, axis=0, keepdims=True)
            outs.append(o * _recip(l))
        out_proj(jnp.maximum(b - 1, 0), o_prev)
        ot = jnp.concatenate(outs, axis=0)
        op_s[...] = _pack(ot.T)

    def attn_last(is_last_layer):
        EQ = 256
        EK = 256
        rbase = (NQ - 1) * TQ

        def proj_piece(o, g, r, cc, final):
            r0 = rbase + r
            cols = slice(cc * 256, (cc + 1) * 256)
            xnew = x[r0:r0 + 128, cols] + _dot(o, wo[1, g * 128:(g + 1) * 128, cols])
            x[r0:r0 + 128, cols] = xnew
            if final:
                xin[r0:r0 + 128, cols] = xnew.astype(BF)
                if cc == 3:
                    @pl.when(is_last_layer)
                    def _():
                        out_copy_last(r // 128).start()

        o_prev = _unpack(op_s[...])
        queue = [(o_prev[r:r + 128, :], G - 2, r, cc, False) for r in range(0, TQ, 128) for cc in range(4)]
        for j in range(TQ // EQ):
            cols = slice(j * EQ, (j + 1) * EQ)
            outs = []
            step = 0
            for hh in range(HPG):
                m = m_buf[hh, :, cols]
                voff = (G - 1) * 64 + hh * 16
                l8 = None
                o = zero_s[:, 0:EQ]
                for c in range(S // EK):
                    p = jnp.exp2(s_buf[hh, c * EK:(c + 1) * EK, cols] - m)
                    for u in range(EK // TK):
                        l8 = lsum(p[u * TK:(u + 1) * TK, :], l8)
                    vc = _unpack(t_s[1, voff:voff + 16, c * EK:(c + 1) * EK])
                    o = o + _dot(vc, p.astype(BF))
                    step += 1
                    if queue and step % 8 in (1, 4, 6):
                        proj_piece(*queue.pop(0))
                l = jnp.sum(l8, axis=0, keepdims=True)
                outs.append(o * _recip(l))
            oj = jnp.concatenate(outs, axis=0).T.astype(BF)
            queue += [(oj[r:r + 128, :], G - 1, j * EQ + r, cc, True) for r in range(0, EQ, 128) for cc in range(4)]
        while queue:
            proj_piece(*queue.pop(0))

    def attention(is_last_layer):
        op_s[...] = jnp.zeros_like(op_s)

        def pro(i, carry):
            for u in range(2):
                hh = 2 * i + u
                qm = get_qm(0, hh)
                m8 = None
                for c in range(NK):
                    m8 = qk_chunk(0, qm, c, hh, m8)
                m_buf[hh] = jnp.max(m8, axis=0, keepdims=True)
            return carry
        with _scope('attn_pro'):
            lax.fori_loop(0, HPG // 2, pro, 0)

        def body(b, carry):
            @pl.when(jnp.logical_and(is_last_layer, jnp.logical_and((b & (G - 1)) == 1, b > G)))
            def _():
                out_copy((b >> 3) - 1).start()
            attn_block(b)
            return carry
        with _scope('attn_loop'):
            lax.fori_loop(0, NBLK - 1, body, 0)
        with _scope('attn_epi'):
            ln0()
            attn_last(is_last_layer)

    with _scope('start'):
        startup()

    def layer(l, carry):
        sel = l & 1
        with _scope('q_phase'):
            q_phase(l)

        @pl.when(l == 0)
        def _():
            for cp in w_copies:
                cp.wait()

        @pl.when(sel == 0)
        def _():
            with _scope('a_mix'):
                a_mix()
            with _scope('a_out'):
                a_out()

        @pl.when(sel == 1)
        def _():
            attention(l == 3)
        return carry

    lax.fori_loop(0, 4, layer, 0)
    for t in range(NTM - 1):
        out_copy(t).wait()
    for j in range(TM // 128):
        out_copy_last(j).wait()


@jax.jit
def pallas_interleave_layers__linear_attn_block__mha_block__prompt_kernel(A_x, A_wqkv, A_wo, B_x, B_wqkv, B_wo):
    del B_x
    scratch = [
        pltpu.VMEM((S, D), BF),
        pltpu.VMEM((S, D), F32),
        pltpu.VMEM((TM // 2, D), U32),
        pltpu.VMEM((TM // 2, D), U32),
        pltpu.VMEM((2, D, 3 * D + WPAD), BF),
        pltpu.VMEM((2, D, D + WPAD), BF),
        pltpu.VMEM((2, D // 2, S), U32),
        pltpu.VMEM((G, S // 2, 128), U32),
        pltpu.VMEM((G, S // 2, 128), U32),
        pltpu.VMEM((TQ // 2, 128), U32),
        pltpu.VMEM((8, D), F32),
        pltpu.VMEM((D // 2, D), U32),
        pltpu.VMEM((DH, TQ), F32),
        pltpu.VMEM((HPG, S, TQ), F32),
        pltpu.VMEM((HPG, 1, TQ), F32),
        pltpu.SemaphoreType.DMA((2,)),
        pltpu.SemaphoreType.DMA((2,)),
        pltpu.SemaphoreType.DMA((1,)),
        pltpu.SemaphoreType.DMA((1,)),
    ]
    out = pl.pallas_call(
        _kernel,
        out_shape=jax.ShapeDtypeStruct((S, D), BF),
        in_specs=[pl.BlockSpec(memory_space=pl.ANY)] * 5,
        out_specs=pl.BlockSpec(memory_space=pl.ANY),
        scratch_shapes=scratch,
        compiler_params=pltpu.CompilerParams(vmem_limit_bytes=120 * 1024 * 1024),
    )(A_x.reshape(S, D), A_wqkv, A_wo, B_wqkv, B_wo)
    return out.reshape(1, S, D)
```

```python
import contextlib
import math

import jax
import jax.numpy as jnp
from jax import lax
import jax.experimental.pallas as pl
import jax.experimental.pallas.tpu as pltpu

S, D, H, DH = 2048, 1024, 32, 32
G = D // 128
HPG = 128 // DH
TM = 512
NTM = S // TM
SUB = 256
TQ = 512
TK = 128
NQ = S // TQ
NK = S // TK
NBLK = G * NQ
PRE = 128
KA = 128
LNC = 32
EPS = 1e-5
WPAD = 256
QSCALE = (DH ** -0.5) * math.log2(math.e)
BF = jnp.bfloat16
F32 = jnp.float32
U32 = jnp.uint32
SCOPES = False


def _scope(name):
    return jax.named_scope(name) if SCOPES else contextlib.nullcontext()


def _pack(v):
    return pltpu.bitcast(v.astype(BF), U32)


def _unpack(u):
    return pltpu.bitcast(u, BF)


def _dot(a, b):
    return jnp.dot(a, b, preferred_element_type=F32)


def _ln(xt):
    mu = jnp.mean(xt, axis=-1, keepdims=True)
    xc = xt - mu
    var = jnp.mean(xc * xc, axis=-1, keepdims=True)
    return (xc * lax.rsqrt(var + EPS)).astype(BF)


def _zero_of(v):
    return pltpu.bitcast(pltpu.bitcast(v, U32) & jnp.uint32(0x80000000), F32)


def _phi(t):
    return jnp.where(t > 0, t + 1.0, jnp.exp(t)) + 1e-6


def _recip(d):
    r = pl.reciprocal(d, approx=True)
    return r * (2.0 - d * r)


def _kernel(x_hbm, wa_hbm, woa_hbm, wb_hbm, wob_hbm, out_hbm,
            xin, x, xn_b, xn_0, wq, wo, t_s, k_s, o_s, op_s, z_acc, m_s, zero_s,
            s_buf, m_buf, sem_x0, sem_wa, sem_w, sem_o):

    XC = S // G

    def x_copy(i):
        r0 = pl.multiple_of(i * XC, XC)
        return pltpu.make_async_copy(x_hbm.at[pl.ds(r0, XC), :], xin.at[pl.ds(r0, XC), :], sem_wa.at[i & 1])

    x0_rows = [(i * 32, 32) for i in range(8)] + [(256 + i * 64, 64) for i in range(4)]
    x0_copies = [pltpu.make_async_copy(x_hbm.at[pl.ds(r, n), :], xin.at[pl.ds(r, n), :], sem_x0.at[i // 8])
                 for i, (r, n) in enumerate(x0_rows)]

    def t_col(j):
        return (1 - (j >> 2)) * (2 * D) + (j & 3) * 256

    def wa_copies(j):
        ct = pl.multiple_of(t_col(j), 256) if not isinstance(j, int) else t_col(j)
        ck = pl.multiple_of(D + j * 128, 128) if not isinstance(j, int) else D + j * 128
        return (pltpu.make_async_copy(wa_hbm.at[:, pl.ds(ct, 256)], wq.at[0, :, pl.ds(ct, 256)], sem_wa.at[j & 1]),
                pltpu.make_async_copy(wa_hbm.at[:, pl.ds(ck, 128)], wq.at[0, :, pl.ds(ck, 128)], sem_wa.at[j & 1]))

    w_copies = [pltpu.make_async_copy(woa_hbm, wo.at[0, :, pl.ds(0, D)], sem_w.at[0]),
                pltpu.make_async_copy(wb_hbm, wq.at[1, :, pl.ds(0, 3 * D)], sem_w.at[0]),
                pltpu.make_async_copy(wob_hbm, wo.at[1, :, pl.ds(0, D)], sem_w.at[0])]

    def out_copy(t):
        return pltpu.make_async_copy(xin.at[pl.ds(t * TM, TM), :], out_hbm.at[pl.ds(t * TM, TM), :], sem_o.at[0])

    def out_copy_last(j):
        r0 = (NTM - 1) * TM + j * 128
        return pltpu.make_async_copy(xin.at[pl.ds(r0, 128), :], out_hbm.at[pl.ds(r0, 128), :],
                                     sem_o.at[0])

    def ln_rows(r0, lo, hi, dep=None):
        paced = dep is not None
        for c in range(lo, hi, LNC):
            xt = x[pl.ds(r0 + c, LNC), :]
            acc = xt[:, 0:128] + dep if paced else xt[:, 0:128]
            for j in range(1, D // 128):
                acc = acc + xt[:, j * 128:(j + 1) * 128]
            mu = jnp.sum(acc, axis=-1, keepdims=True) * (1.0 / D)
            xc = xt - mu
            var = jnp.mean(xc * xc, axis=-1, keepdims=True)
            r = lax.rsqrt(var + EPS)
            xn_b[c // 2:(c + LNC) // 2, :] = _pack(xc * r)
            dep = _zero_of(r)
        return dep

    def ln0():
        ln_rows(0, 0, PRE)

    def q_phase(l):
        sel = l & 1
        is_a = sel == 0
        first = l == 0

        def k_part(t, lo, hi, xn, c0, cn):
            rh = pl.multiple_of(t * (TM // 2) + lo // 2, 64)
            k = _dot(xn, wq[sel, :, D + c0:D + c0 + cn])
            kk = jnp.where(is_a, _phi(k), k)
            z_acc[:, c0:c0 + cn] += jnp.sum(kk.reshape((hi - lo) // 8, 8, cn), axis=0)
            kb = _pack(kk)
            for g in range(cn // 128):
                k_s[c0 // 128 + g, pl.ds(rh, (hi - lo) // 2), :] = kb[:, g * 128:(g + 1) * 128]

        def body(t, carry):
            rt = pl.multiple_of(t * TM, TM)
            rn = pl.multiple_of(jnp.minimum(t + 1, NTM - 1) * TM, TM)
            ln_rows(rt, PRE, TM)
            xn_all = _unpack(xn_b[...])
            for lo, hi in ((0, PRE), (PRE, TM)):
                v = _dot(xn_all[lo:hi, :], wq[sel, :, 2 * D:3 * D])
                t_s[1, :, pl.ds(rt + lo, hi - lo)] = _pack(v.T)
            for sb in range(TM // SUB):
                r0 = pl.multiple_of(t * TM + sb * SUB, SUB)
                xn = xn_all[sb * SUB:(sb + 1) * SUB, :]
                q = _dot(xn, wq[sel, :, 0:D]).T
                qq = jnp.where(is_a, _phi(q), q * QSCALE)
                t_s[0, :, pl.ds(r0, SUB)] = _pack(qq)
                if sb == 0:
                    dep = _zero_of(qq[0:LNC, 0:128])
            ln_rows(rn, 0, PRE, dep)
            for sb in range(TM // SUB):
                k_part(t, sb * SUB, (sb + 1) * SUB, xn_all[sb * SUB:(sb + 1) * SUB, :], 0, D)
            return carry

        @pl.when(l > 0)
        def _():
            z_acc[...] = jnp.zeros_like(z_acc)
        lax.fori_loop(jnp.where(first, 1, 0), NTM, body, 0)

    def startup():
        for cp in x0_copies:
            cp.start()
        for cp in wa_copies(0):
            cp.start()
        zero_s[...] = jnp.zeros_like(zero_s)
        for cp in x0_copies[:8]:
            cp.wait()
        xn_0[0:128, :] = _pack(_ln(xin[0:256, :].astype(F32)))
        for cp in x0_copies[8:]:
            cp.wait()
        xn_0[128:256, :] = _pack(_ln(xin[256:512, :].astype(F32)))
        for cp in wa_copies(1):
            cp.start()
        for cp in wa_copies(0):
            cp.wait()

        def body(j, carry):
            xn = _unpack(xn_0[...])
            ct = pl.multiple_of(t_col(j), 256)
            ck = pl.multiple_of(j * 128, 128)
            rc = pl.multiple_of(j * XC, XC)
            xf = xin[pl.ds(rc, XC), :].astype(F32)
            x[pl.ds(rc, XC), :] = xf
            u = pltpu.bitcast(xf, U32)
            u = u[:, 0:512] | u[:, 512:1024]
            u = jnp.concatenate([u[:, 0:256], u[:, 256:512]], axis=0) & jnp.uint32(0x80000000)
            y = (_dot(xn, wq[0, :, pl.ds(ct, 256)]) + pltpu.bitcast(u, F32)).T
            y = jnp.where(j >= 4, _phi(y), y)
            tr = pl.multiple_of((j & 3) * 128, 128)
            t_s[1 - (j >> 2), pl.ds(tr, 128), 0:TM] = _pack(y)
            kk = _phi(_dot(xn, wq[0, :, pl.ds(D + ck, 128)]))
            z_acc[:, pl.ds(ck, 128)] = jnp.sum(kk.reshape(TM // 8, 8, 128), axis=0)
            k_s[j, 0:TM // 2, :] = _pack(kk)

            @pl.when(j + 2 < G)
            def _():
                x_copy(j + 2).start()
                for cp in wa_copies(j + 2):
                    cp.start()

            @pl.when(j == G - 2)
            def _():
                for cp in w_copies:
                    cp.start()

            @pl.when(j + 1 < G)
            def _():
                for cp in wa_copies(j + 1):
                    cp.wait()

                @pl.when(j > 0)
                def _():
                    x_copy(j + 1).wait()
            return carry
        lax.fori_loop(0, G, body, 0)
        ln_rows(TM, 0, PRE)

    def a_mix():
        row = lax.broadcasted_iota(jnp.int32, (128, 128), 0) // DH
        col = lax.broadcasted_iota(jnp.int32, (128, 128), 1) // DH
        same = row == col
        zrow = lax.broadcasted_iota(jnp.int32, (16, 128), 0)
        zcol = lax.broadcasted_iota(jnp.int32, (16, 128), 1) // DH
        zsel = zrow == zcol
        z = jnp.sum(z_acc[...], axis=0, keepdims=True)

        def fold(g, kvg):
            m_s[g * 64:(g + 1) * 64, :] = _pack(_dot(kvg, wo[0, g * 128:(g + 1) * 128, 0:D]))

        def group(g):
            zg = jnp.broadcast_to(z[:, g * 128:(g + 1) * 128], (16, 128))
            zl = jnp.where(zsel, zg, 0.0).astype(BF)
            kvt = None
            for t in range(NTM):
                pqt = _unpack(t_s[0, g * 64:(g + 1) * 64, t * TM:(t + 1) * TM])
                r = _recip(_dot(zl, pqt)[0:8, :] + 1e-6)
                pf = pqt.astype(F32)
                ot = jnp.concatenate(
                    [pf[j * DH:(j + 1) * DH, :] * r[j:j + 1, :] for j in range(HPG)], axis=0)
                o_s[g, t * TM // 2:(t + 1) * TM // 2, :] = _pack(ot.T)
                part = _dot(_unpack(t_s[1, g * 64:(g + 1) * 64, t * TM:(t + 1) * TM]),
                            _unpack(k_s[g, t * TM // 2:(t + 1) * TM // 2, :]))
                kvt = part if kvt is None else kvt + part
            return jnp.where(same, kvt, 0.0).T.astype(BF)

        kvs = []
        for g in range(G):
            kvs.append(group(g))
            if g >= 2:
                fold(g - 2, kvs[g - 2])
        fold(G - 2, kvs[G - 2])
        fold(G - 1, kvs[G - 1])

    def a_out():
        def body(t, carry):
            for sb in range(TM // SUB):
                r0 = pl.multiple_of(t * TM + sb * SUB, SUB)
                rh = pl.multiple_of(t * (TM // 2) + sb * (SUB // 2), SUB // 2)
                o = jnp.concatenate([_unpack(o_s[g, pl.ds(rh, SUB // 2), :]) for g in range(G)], axis=1)
                xnew = x[pl.ds(r0, SUB), :] + _dot(o, _unpack(m_s[...]))
                x[pl.ds(r0, SUB), :] = xnew
                if sb == 0:
                    dep = None
                    for c in range(0, PRE, LNC):
                        xt = xnew[c:c + LNC, :]
                        acc = xt[:, 0:128] if dep is None else xt[:, 0:128] + dep
                        for j in range(1, D // 128):
                            acc = acc + xt[:, j * 128:(j + 1) * 128]
                        mu = jnp.sum(acc, axis=-1, keepdims=True) * (1.0 / D)
                        xc = xt - mu
                        var = jnp.mean(xc * xc, axis=-1, keepdims=True)
                        r = lax.rsqrt(var + EPS)
                        rows = slice(c // 2, (c + LNC) // 2)
                        xn_b[rows, :] = jnp.where(t == 0, _pack(xc * r), xn_b[rows, :])
                        if False:
                            dep = _zero_of(r)
            return carry
        lax.fori_loop(0, NTM, body, 0)

    def decode(b):
        return b & (G - 1), b >> 3

    def get_qm(b, hh):
        g, qi = decode(b)
        qoff = pl.multiple_of(qi * TQ, TQ)
        if isinstance(hh, int):
            roff = pl.multiple_of(g * 64 + hh * 16, 16)
            parts = []
            if hh > 0:
                parts.append(jnp.zeros((hh * 16, TQ), U32))
            parts.append(t_s[0, pl.ds(roff, 16), pl.ds(qoff, TQ)])
            if hh < HPG - 1:
                parts.append(jnp.zeros(((HPG - 1 - hh) * 16, TQ), U32))
            return _unpack(jnp.concatenate(parts, axis=0))
        roff = pl.multiple_of(g * 64, 64)
        qg = t_s[0, pl.ds(roff, 64), pl.ds(qoff, TQ)]
        row = lax.broadcasted_iota(jnp.int32, (64, TQ), 0) // 16
        return _unpack(jnp.where(row == hh, qg, jnp.zeros_like(qg)))

    def qk_chunk(g, qm, c, hh, m8):
        kc = _unpack(k_s[g, c * TK // 2:(c + 1) * TK // 2, :])
        s = _dot(kc, qm)
        s_buf[hh, c * TK:(c + 1) * TK, :] = s
        mc = jnp.max(s.reshape(TK // 8, 8, TQ), axis=0)
        return mc if m8 is None else jnp.maximum(m8, mc)

    def out_proj(b, o):
        g, qi = decode(b)
        r0 = pl.multiple_of(qi * TQ, TQ)
        w0 = pl.multiple_of(g * 128, 128)
        xnew = x[pl.ds(r0, TQ), :] + _dot(o, wo[1, pl.ds(w0, 128), 0:D])
        x[pl.ds(r0, TQ), :] = xnew
        xin[pl.ds(r0, TQ), :] = xnew.astype(BF)

    def lsum(p, l8):
        for r in range(TK // 16 - 1, -1, -1):
            pr = p[r * 16:r * 16 + 8, :] + p[r * 16 + 8:r * 16 + 16, :]
            l8 = pr if l8 is None else l8 + pr
        return l8

    def attn_block(b):
        gc, qi = decode(b)
        gn = (b + 1) & (G - 1)
        o_prev = _unpack(op_s[...])
        outs = []
        ms = [m_buf[hh] for hh in range(HPG)]
        for hh in range(HPG):
            qm = get_qm(b + 1, hh)
            voff = pl.multiple_of(gc * 64 + hh * 16, 16)
            l8 = None
            o = zero_s[...]
            m8 = None
            for c in range(NK):
                p = jnp.exp2(s_buf[hh, c * TK:(c + 1) * TK, :] - ms[hh])
                l8 = lsum(p, l8)
                m8 = qk_chunk(gn, qm, c, hh, m8)
                vc = _unpack(t_s[1, pl.ds(voff, 16), c * TK:(c + 1) * TK])
                o = o + _dot(vc, p.astype(BF))
            m_buf[hh] = jnp.max(m8, axis=0, keepdims=True)
            l = jnp.sum(l8, axis=0, keepdims=True)
            outs.append(o * _recip(l))
        out_proj(jnp.maximum(b - 1, 0), o_prev)
        ot = jnp.concatenate(outs, axis=0)
        op_s[...] = _pack(ot.T)

    def attn_last(is_last_layer):
        EQ = 256
        EK = 256
        rbase = (NQ - 1) * TQ

        def proj_piece(o, g, r, cc, final):
            r0 = rbase + r
            cols = slice(cc * 256, (cc + 1) * 256)
            xnew = x[r0:r0 + 128, cols] + _dot(o, wo[1, g * 128:(g + 1) * 128, cols])
            x[r0:r0 + 128, cols] = xnew
            if final:
                xin[r0:r0 + 128, cols] = xnew.astype(BF)
                if cc == 3:
                    @pl.when(is_last_layer)
                    def _():
                        out_copy_last(r // 128).start()

        o_prev = _unpack(op_s[...])
        queue = [(o_prev[r:r + 128, :], G - 2, r, cc, False) for r in range(0, TQ, 128) for cc in range(4)]
        for j in range(TQ // EQ):
            cols = slice(j * EQ, (j + 1) * EQ)
            outs = []
            step = 0
            for hh in range(HPG):
                m = m_buf[hh, :, cols]
                voff = (G - 1) * 64 + hh * 16
                l8 = None
                o = zero_s[:, 0:EQ]
                for c in range(S // EK):
                    p = jnp.exp2(s_buf[hh, c * EK:(c + 1) * EK, cols] - m)
                    for u in range(EK // TK):
                        l8 = lsum(p[u * TK:(u + 1) * TK, :], l8)
                    vc = _unpack(t_s[1, voff:voff + 16, c * EK:(c + 1) * EK])
                    o = o + _dot(vc, p.astype(BF))
                    step += 1
                    if queue and step % 8 in (1, 4, 6):
                        proj_piece(*queue.pop(0))
                l = jnp.sum(l8, axis=0, keepdims=True)
                outs.append(o * _recip(l))
            oj = jnp.concatenate(outs, axis=0).T.astype(BF)
            queue += [(oj[r:r + 128, :], G - 1, j * EQ + r, cc, True) for r in range(0, EQ, 128) for cc in range(4)]
        while queue:
            proj_piece(*queue.pop(0))

    def attention(is_last_layer):
        op_s[...] = jnp.zeros_like(op_s)

        def pro(i, carry):
            for u in range(2):
                hh = 2 * i + u
                qm = get_qm(0, hh)
                m8 = None
                for c in range(NK):
                    m8 = qk_chunk(0, qm, c, hh, m8)
                m_buf[hh] = jnp.max(m8, axis=0, keepdims=True)
            return carry
        with _scope('attn_pro'):
            lax.fori_loop(0, HPG // 2, pro, 0)

        def body(b, carry):
            @pl.when(jnp.logical_and(is_last_layer, jnp.logical_and((b & (G - 1)) == 1, b > G)))
            def _():
                out_copy((b >> 3) - 1).start()
            attn_block(b)
            return carry
        with _scope('attn_loop'):
            lax.fori_loop(0, NBLK - 1, body, 0)
        with _scope('attn_epi'):
            ln0()
            attn_last(is_last_layer)

    with _scope('start'):
        startup()

    def layer(l, carry):
        sel = l & 1
        with _scope('q_phase'):
            q_phase(l)

        @pl.when(l == 0)
        def _():
            for cp in w_copies:
                cp.wait()

        @pl.when(sel == 0)
        def _():
            with _scope('a_mix'):
                a_mix()
            with _scope('a_out'):
                a_out()

        @pl.when(sel == 1)
        def _():
            attention(l == 3)
        return carry

    lax.fori_loop(0, 4, layer, 0)
    for t in range(NTM - 1):
        out_copy(t).wait()
    for j in range(TM // 128):
        out_copy_last(j).wait()


@jax.jit
def pallas_interleave_layers__linear_attn_block__mha_block__prompt_kernel(A_x, A_wqkv, A_wo, B_x, B_wqkv, B_wo):
    del B_x
    scratch = [
        pltpu.VMEM((S, D), BF),
        pltpu.VMEM((S, D), F32),
        pltpu.VMEM((TM // 2, D), U32),
        pltpu.VMEM((TM // 2, D), U32),
        pltpu.VMEM((2, D, 3 * D + WPAD), BF),
        pltpu.VMEM((2, D, D + WPAD), BF),
        pltpu.VMEM((2, D // 2, S), U32),
        pltpu.VMEM((G, S // 2, 128), U32),
        pltpu.VMEM((G, S // 2, 128), U32),
        pltpu.VMEM((TQ // 2, 128), U32),
        pltpu.VMEM((8, D), F32),
        pltpu.VMEM((D // 2, D), U32),
        pltpu.VMEM((DH, TQ), F32),
        pltpu.VMEM((HPG, S, TQ), F32),
        pltpu.VMEM((HPG, 1, TQ), F32),
        pltpu.SemaphoreType.DMA((2,)),
        pltpu.SemaphoreType.DMA((2,)),
        pltpu.SemaphoreType.DMA((1,)),
        pltpu.SemaphoreType.DMA((1,)),
    ]
    out = pl.pallas_call(
        _kernel,
        out_shape=jax.ShapeDtypeStruct((S, D), BF),
        in_specs=[pl.BlockSpec(memory_space=pl.ANY)] * 5,
        out_specs=pl.BlockSpec(memory_space=pl.ANY),
        scratch_shapes=scratch,
        compiler_params=pltpu.CompilerParams(vmem_limit_bytes=120 * 1024 * 1024, disable_bounds_checks=True, disable_semaphore_checks=True),
    )(A_x.reshape(S, D), A_wqkv, A_wo, B_wqkv, B_wo)
    return out.reshape(1, S, D)
```

```python
import math

import jax
import jax.numpy as jnp
from jax import lax
import jax.experimental.pallas as pl
import jax.experimental.pallas.tpu as pltpu

S, D, H, DH = 2048, 1024, 32, 32
G = D // 128
HPG = 128 // DH
TM = 512
NTM = S // TM
SUB = 256
TQ = 512
TK = 128
NQ = S // TQ
NK = S // TK
NBLK = G * NQ
PRE = 128
LNC = 32
XC = S // G
EPS = 1e-5
WPAD = 256
QSCALE = (DH ** -0.5) * math.log2(math.e)
BF = jnp.bfloat16
F32 = jnp.float32
U32 = jnp.uint32


def _pack(v):
    return pltpu.bitcast(v.astype(BF), U32)


def _unpack(u):
    return pltpu.bitcast(u, BF)


def _dot(a, b):
    return jnp.dot(a, b, preferred_element_type=F32)


def _ln(xt):
    mu = jnp.mean(xt, axis=-1, keepdims=True)
    xc = xt - mu
    var = jnp.mean(xc * xc, axis=-1, keepdims=True)
    return (xc * lax.rsqrt(var + EPS)).astype(BF)


def _ln_chunk(xt, dep=None):
    acc = xt[:, 0:128] if dep is None else xt[:, 0:128] + dep
    for j in range(1, D // 128):
        acc = acc + xt[:, j * 128:(j + 1) * 128]
    mu = jnp.sum(acc, axis=-1, keepdims=True) * (1.0 / D)
    xc = xt - mu
    var = jnp.mean(xc * xc, axis=-1, keepdims=True)
    r = lax.rsqrt(var + EPS)
    return xc * r, r


def _zero_of(v):
    return pltpu.bitcast(pltpu.bitcast(v, U32) & jnp.uint32(0x80000000), F32)


def _phi(t):
    return jnp.where(t > 0, t + 1.0, jnp.exp(t)) + 1e-6


def _recip(d):
    r = pl.reciprocal(d, approx=True)
    return r * (2.0 - d * r)


def _kernel(x_hbm, wa_hbm, woa_hbm, wb_hbm, wob_hbm, out_hbm,
            xin, x, xn_b, xn_0, wq, wo, t_s, k_s, o_s, op_s, z_acc, m_s, zero_s,
            s_buf, m_buf, sem_x0, sem_wa, sem_w, sem_o):

    def x_copy(i):
        r0 = pl.multiple_of(i * XC, XC)
        return pltpu.make_async_copy(x_hbm.at[pl.ds(r0, XC), :], xin.at[pl.ds(r0, XC), :], sem_wa.at[i & 1])

    x0_rows = [(i * 32, 32) for i in range(8)] + [(256 + i * 64, 64) for i in range(4)]
    x0_copies = [pltpu.make_async_copy(x_hbm.at[pl.ds(r, n), :], xin.at[pl.ds(r, n), :], sem_x0.at[i // 8])
                 for i, (r, n) in enumerate(x0_rows)]

    def t_col(j):
        return (1 - (j >> 2)) * (2 * D) + (j & 3) * 256

    def wa_copies(j):
        ct = pl.multiple_of(t_col(j), 256) if not isinstance(j, int) else t_col(j)
        ck = pl.multiple_of(D + j * 128, 128) if not isinstance(j, int) else D + j * 128
        return (pltpu.make_async_copy(wa_hbm.at[:, pl.ds(ct, 256)], wq.at[0, :, pl.ds(ct, 256)], sem_wa.at[j & 1]),
                pltpu.make_async_copy(wa_hbm.at[:, pl.ds(ck, 128)], wq.at[0, :, pl.ds(ck, 128)], sem_wa.at[j & 1]))

    w_copies = [pltpu.make_async_copy(woa_hbm, wo.at[0, :, pl.ds(0, D)], sem_w.at[0]),
                pltpu.make_async_copy(wb_hbm, wq.at[1, :, pl.ds(0, 3 * D)], sem_w.at[0]),
                pltpu.make_async_copy(wob_hbm, wo.at[1, :, pl.ds(0, D)], sem_w.at[0])]

    def out_copy(t):
        return pltpu.make_async_copy(xin.at[pl.ds(t * TM, TM), :], out_hbm.at[pl.ds(t * TM, TM), :], sem_o.at[0])

    def out_copy_last(j):
        r0 = (NTM - 1) * TM + j * 128
        return pltpu.make_async_copy(xin.at[pl.ds(r0, 128), :], out_hbm.at[pl.ds(r0, 128), :], sem_o.at[0])

    def ln_rows(r0, lo, hi, dep=None):
        for c in range(lo, hi, LNC):
            xn, r = _ln_chunk(x[pl.ds(r0 + c, LNC), :], dep)
            xn_b[c // 2:(c + LNC) // 2, :] = _pack(xn)
            if dep is not None:
                dep = _zero_of(r)

    def q_phase(l):
        sel = l & 1
        is_a = sel == 0

        def body(t, carry):
            rt = pl.multiple_of(t * TM, TM)
            rn = pl.multiple_of(jnp.minimum(t + 1, NTM - 1) * TM, TM)
            ln_rows(rt, PRE, TM)
            xn_all = _unpack(xn_b[...])
            for lo, hi in ((0, PRE), (PRE, TM)):
                v = _dot(xn_all[lo:hi, :], wq[sel, :, 2 * D:3 * D])
                t_s[1, :, pl.ds(rt + lo, hi - lo)] = _pack(v.T)
            for sb in range(TM // SUB):
                r0 = pl.multiple_of(t * TM + sb * SUB, SUB)
                xn = xn_all[sb * SUB:(sb + 1) * SUB, :]
                q = _dot(xn, wq[sel, :, 0:D]).T
                qq = jnp.where(is_a, _phi(q), q * QSCALE)
                t_s[0, :, pl.ds(r0, SUB)] = _pack(qq)
                if sb == 0:
                    dep = _zero_of(qq[0:LNC, 0:128])
            ln_rows(rn, 0, PRE, dep)
            for sb in range(TM // SUB):
                rh = pl.multiple_of(t * (TM // 2) + sb * (SUB // 2), 64)
                k = _dot(xn_all[sb * SUB:(sb + 1) * SUB, :], wq[sel, :, D:2 * D])
                kk = jnp.where(is_a, _phi(k), k)
                z_acc[...] += jnp.sum(kk.reshape(SUB // 8, 8, D), axis=0)
                kb = _pack(kk)
                for g in range(G):
                    k_s[g, pl.ds(rh, SUB // 2), :] = kb[:, g * 128:(g + 1) * 128]
            return carry

        @pl.when(l > 0)
        def _():
            z_acc[...] = jnp.zeros_like(z_acc)
        lax.fori_loop(jnp.where(l == 0, 1, 0), NTM, body, 0)

    def startup():
        for cp in x0_copies:
            cp.start()
        for cp in wa_copies(0):
            cp.start()
        zero_s[...] = jnp.zeros_like(zero_s)
        for cp in x0_copies[:8]:
            cp.wait()
        xn_0[0:128, :] = _pack(_ln(xin[0:256, :].astype(F32)))
        for cp in x0_copies[8:]:
            cp.wait()
        xn_0[128:256, :] = _pack(_ln(xin[256:512, :].astype(F32)))
        for cp in wa_copies(1):
            cp.start()
        for cp in wa_copies(0):
            cp.wait()

        def body(j, carry):
            xn = _unpack(xn_0[...])
            ct = pl.multiple_of(t_col(j), 256)
            ck = pl.multiple_of(j * 128, 128)
            rc = pl.multiple_of(j * XC, XC)
            xf = xin[pl.ds(rc, XC), :].astype(F32)
            x[pl.ds(rc, XC), :] = xf
            u = pltpu.bitcast(xf, U32)
            u = u[:, 0:512] | u[:, 512:1024]
            u = jnp.concatenate([u[:, 0:256], u[:, 256:512]], axis=0) & jnp.uint32(0x80000000)
            y = (_dot(xn, wq[0, :, pl.ds(ct, 256)]) + pltpu.bitcast(u, F32)).T
            y = jnp.where(j >= 4, _phi(y), y)
            tr = pl.multiple_of((j & 3) * 128, 128)
            t_s[1 - (j >> 2), pl.ds(tr, 128), 0:TM] = _pack(y)
            kk = _phi(_dot(xn, wq[0, :, pl.ds(D + ck, 128)]))
            z_acc[:, pl.ds(ck, 128)] = jnp.sum(kk.reshape(TM // 8, 8, 128), axis=0)
            k_s[j, 0:TM // 2, :] = _pack(kk)

            @pl.when(j + 2 < G)
            def _():
                x_copy(j + 2).start()
                for cp in wa_copies(j + 2):
                    cp.start()

            @pl.when(j == G - 2)
            def _():
                for cp in w_copies:
                    cp.start()

            @pl.when(j + 1 < G)
            def _():
                for cp in wa_copies(j + 1):
                    cp.wait()

                @pl.when(j > 0)
                def _():
                    x_copy(j + 1).wait()
            return carry
        lax.fori_loop(0, G, body, 0)
        ln_rows(TM, 0, PRE)

    def a_mix():
        row = lax.broadcasted_iota(jnp.int32, (128, 128), 0) // DH
        col = lax.broadcasted_iota(jnp.int32, (128, 128), 1) // DH
        same = row == col
        zrow = lax.broadcasted_iota(jnp.int32, (16, 128), 0)
        zcol = lax.broadcasted_iota(jnp.int32, (16, 128), 1) // DH
        zsel = zrow == zcol
        z = jnp.sum(z_acc[...], axis=0, keepdims=True)

        def fold(g, kvg):
            m_s[g * 64:(g + 1) * 64, :] = _pack(_dot(kvg, wo[0, g * 128:(g + 1) * 128, 0:D]))

        def group(g):
            zg = jnp.broadcast_to(z[:, g * 128:(g + 1) * 128], (16, 128))
            zl = jnp.where(zsel, zg, 0.0).astype(BF)
            kvt = None
            for t in range(NTM):
                pqt = _unpack(t_s[0, g * 64:(g + 1) * 64, t * TM:(t + 1) * TM])
                r = _recip(_dot(zl, pqt)[0:8, :] + 1e-6)
                pf = pqt.astype(F32)
                ot = jnp.concatenate(
                    [pf[j * DH:(j + 1) * DH, :] * r[j:j + 1, :] for j in range(HPG)], axis=0)
                o_s[g, t * TM // 2:(t + 1) * TM // 2, :] = _pack(ot.T)
                part = _dot(_unpack(t_s[1, g * 64:(g + 1) * 64, t * TM:(t + 1) * TM]),
                            _unpack(k_s[g, t * TM // 2:(t + 1) * TM // 2, :]))
                kvt = part if kvt is None else kvt + part
            return jnp.where(same, kvt, 0.0).T.astype(BF)

        kvs = []
        for g in range(G):
            kvs.append(group(g))
            if g >= 2:
                fold(g - 2, kvs[g - 2])
        fold(G - 2, kvs[G - 2])
        fold(G - 1, kvs[G - 1])

    def a_out():
        def body(t, carry):
            for sb in range(TM // SUB):
                r0 = pl.multiple_of(t * TM + sb * SUB, SUB)
                rh = pl.multiple_of(t * (TM // 2) + sb * (SUB // 2), SUB // 2)
                o = jnp.concatenate([_unpack(o_s[g, pl.ds(rh, SUB // 2), :]) for g in range(G)], axis=1)
                xnew = x[pl.ds(r0, SUB), :] + _dot(o, _unpack(m_s[...]))
                x[pl.ds(r0, SUB), :] = xnew
                if sb == 0:
                    for c in range(0, PRE, LNC):
                        xn, _ = _ln_chunk(xnew[c:c + LNC, :])
                        rows = slice(c // 2, (c + LNC) // 2)
                        xn_b[rows, :] = jnp.where(t == 0, _pack(xn), xn_b[rows, :])
            return carry
        lax.fori_loop(0, NTM, body, 0)

    def decode(b):
        return b & (G - 1), b >> 3

    def get_qm(b, hh):
        g, qi = decode(b)
        qoff = pl.multiple_of(qi * TQ, TQ)
        if isinstance(hh, int):
            roff = pl.multiple_of(g * 64 + hh * 16, 16)
            parts = []
            if hh > 0:
                parts.append(jnp.zeros((hh * 16, TQ), U32))
            parts.append(t_s[0, pl.ds(roff, 16), pl.ds(qoff, TQ)])
            if hh < HPG - 1:
                parts.append(jnp.zeros(((HPG - 1 - hh) * 16, TQ), U32))
            return _unpack(jnp.concatenate(parts, axis=0))
        roff = pl.multiple_of(g * 64, 64)
        qg = t_s[0, pl.ds(roff, 64), pl.ds(qoff, TQ)]
        row = lax.broadcasted_iota(jnp.int32, (64, TQ), 0) // 16
        return _unpack(jnp.where(row == hh, qg, jnp.zeros_like(qg)))

    def qk_chunk(g, qm, c, hh, m8):
        kc = _unpack(k_s[g, c * TK // 2:(c + 1) * TK // 2, :])
        s = _dot(kc, qm)
        s_buf[hh, c * TK:(c + 1) * TK, :] = s
        mc = jnp.max(s.reshape(TK // 8, 8, TQ), axis=0)
        return mc if m8 is None else jnp.maximum(m8, mc)

    def out_proj(b, o):
        g, qi = decode(b)
        r0 = pl.multiple_of(qi * TQ, TQ)
        w0 = pl.multiple_of(g * 128, 128)
        xnew = x[pl.ds(r0, TQ), :] + _dot(o, wo[1, pl.ds(w0, 128), 0:D])
        x[pl.ds(r0, TQ), :] = xnew
        xin[pl.ds(r0, TQ), :] = xnew.astype(BF)

    def lsum(p, l8):
        for r in range(TK // 16 - 1, -1, -1):
            pr = p[r * 16:r * 16 + 8, :] + p[r * 16 + 8:r * 16 + 16, :]
            l8 = pr if l8 is None else l8 + pr
        return l8

    def attn_block(b):
        gc, _ = decode(b)
        gn = (b + 1) & (G - 1)
        o_prev = _unpack(op_s[...])
        outs = []
        ms = [m_buf[hh] for hh in range(HPG)]
        for hh in range(HPG):
            qm = get_qm(b + 1, hh)
            voff = pl.multiple_of(gc * 64 + hh * 16, 16)
            l8 = None
            o = zero_s[...]
            m8 = None
            for c in range(NK):
                p = jnp.exp2(s_buf[hh, c * TK:(c + 1) * TK, :] - ms[hh])
                l8 = lsum(p, l8)
                m8 = qk_chunk(gn, qm, c, hh, m8)
                vc = _unpack(t_s[1, pl.ds(voff, 16), c * TK:(c + 1) * TK])
                o = o + _dot(vc, p.astype(BF))
            m_buf[hh] = jnp.max(m8, axis=0, keepdims=True)
            l = jnp.sum(l8, axis=0, keepdims=True)
            outs.append(o * _recip(l))
        out_proj(jnp.maximum(b - 1, 0), o_prev)
        ot = jnp.concatenate(outs, axis=0)
        op_s[...] = _pack(ot.T)

    def attn_last(is_last_layer):
        EQ = 256
        EK = 256
        rbase = (NQ - 1) * TQ

        def proj_piece(o, g, r, cc, final):
            r0 = rbase + r
            cols = slice(cc * 256, (cc + 1) * 256)
            xnew = x[r0:r0 + 128, cols] + _dot(o, wo[1, g * 128:(g + 1) * 128, cols])
            x[r0:r0 + 128, cols] = xnew
            if final:
                xin[r0:r0 + 128, cols] = xnew.astype(BF)
                if cc == 3:
                    @pl.when(is_last_layer)
                    def _():
                        out_copy_last(r // 128).start()

        o_prev = _unpack(op_s[...])
        queue = [(o_prev[r:r + 128, :], G - 2, r, cc, False) for r in range(0, TQ, 128) for cc in range(4)]
        for j in range(TQ // EQ):
            cols = slice(j * EQ, (j + 1) * EQ)
            outs = []
            step = 0
            for hh in range(HPG):
                m = m_buf[hh, :, cols]
                voff = (G - 1) * 64 + hh * 16
                l8 = None
                o = zero_s[:, 0:EQ]
                for c in range(S // EK):
                    p = jnp.exp2(s_buf[hh, c * EK:(c + 1) * EK, cols] - m)
                    for u in range(EK // TK):
                        l8 = lsum(p[u * TK:(u + 1) * TK, :], l8)
                    vc = _unpack(t_s[1, voff:voff + 16, c * EK:(c + 1) * EK])
                    o = o + _dot(vc, p.astype(BF))
                    step += 1
                    if queue and step % 8 in (1, 4, 6):
                        proj_piece(*queue.pop(0))
                l = jnp.sum(l8, axis=0, keepdims=True)
                outs.append(o * _recip(l))
            oj = jnp.concatenate(outs, axis=0).T.astype(BF)
            queue += [(oj[r:r + 128, :], G - 1, j * EQ + r, cc, True) for r in range(0, EQ, 128) for cc in range(4)]
        while queue:
            proj_piece(*queue.pop(0))

    def attention(is_last_layer):
        op_s[...] = jnp.zeros_like(op_s)

        def pro(i, carry):
            for u in range(2):
                hh = 2 * i + u
                qm = get_qm(0, hh)
                m8 = None
                for c in range(NK):
                    m8 = qk_chunk(0, qm, c, hh, m8)
                m_buf[hh] = jnp.max(m8, axis=0, keepdims=True)
            return carry
        lax.fori_loop(0, HPG // 2, pro, 0)

        def body(b, carry):
            @pl.when(jnp.logical_and(is_last_layer, jnp.logical_and((b & (G - 1)) == 1, b > G)))
            def _():
                out_copy((b >> 3) - 1).start()
            attn_block(b)
            return carry
        lax.fori_loop(0, NBLK - 1, body, 0)
        ln_rows(0, 0, PRE)
        attn_last(is_last_layer)

    startup()

    def layer(l, carry):
        sel = l & 1
        q_phase(l)

        @pl.when(l == 0)
        def _():
            for cp in w_copies:
                cp.wait()

        @pl.when(sel == 0)
        def _():
            a_mix()
            a_out()

        @pl.when(sel == 1)
        def _():
            attention(l == 3)
        return carry

    lax.fori_loop(0, 4, layer, 0)
    for t in range(NTM - 1):
        out_copy(t).wait()
    for j in range(TM // 128):
        out_copy_last(j).wait()


@jax.jit
def pallas_interleave_layers__linear_attn_block__mha_block__prompt_kernel(A_x, A_wqkv, A_wo, B_x, B_wqkv, B_wo):
    del B_x
    scratch = [
        pltpu.VMEM((S, D), BF),
        pltpu.VMEM((S, D), F32),
        pltpu.VMEM((TM // 2, D), U32),
        pltpu.VMEM((TM // 2, D), U32),
        pltpu.VMEM((2, D, 3 * D + WPAD), BF),
        pltpu.VMEM((2, D, D + WPAD), BF),
        pltpu.VMEM((2, D // 2, S), U32),
        pltpu.VMEM((G, S // 2, 128), U32),
        pltpu.VMEM((G, S // 2, 128), U32),
        pltpu.VMEM((TQ // 2, 128), U32),
        pltpu.VMEM((8, D), F32),
        pltpu.VMEM((D // 2, D), U32),
        pltpu.VMEM((DH, TQ), F32),
        pltpu.VMEM((HPG, S, TQ), F32),
        pltpu.VMEM((HPG, 1, TQ), F32),
        pltpu.SemaphoreType.DMA((2,)),
        pltpu.SemaphoreType.DMA((2,)),
        pltpu.SemaphoreType.DMA((1,)),
        pltpu.SemaphoreType.DMA((1,)),
    ]
    out = pl.pallas_call(
        _kernel,
        out_shape=jax.ShapeDtypeStruct((S, D), BF),
        in_specs=[pl.BlockSpec(memory_space=pl.ANY)] * 5,
        out_specs=pl.BlockSpec(memory_space=pl.ANY),
        scratch_shapes=scratch,
        compiler_params=pltpu.CompilerParams(
            vmem_limit_bytes=120 * 1024 * 1024,
            disable_bounds_checks=True,
            disable_semaphore_checks=True,
        ),
    )(A_x.reshape(S, D), A_wqkv, A_wo, B_wqkv, B_wo)
    return out.reshape(1, S, D)
```

```python
import math

import jax
import jax.numpy as jnp
from jax import lax
import jax.experimental.pallas as pl
import jax.experimental.pallas.tpu as pltpu

S, D, H, DH = 2048, 1024, 32, 32
G = D // 128
HPG = 128 // DH
TM = 512
NTM = S // TM
SUB = 256
TQ = 512
TK = 128
NQ = S // TQ
NK = S // TK
NBLK = G * NQ
PRE = 128
LNC = 32
XC = S // G
EPS = 1e-5
WPAD = 256
QSCALE = (DH ** -0.5) * math.log2(math.e)
BF = jnp.bfloat16
F32 = jnp.float32
U32 = jnp.uint32


def _pack(v):
    return pltpu.bitcast(v.astype(BF), U32)


def _unpack(u):
    return pltpu.bitcast(u, BF)


def _dot(a, b):
    return jnp.dot(a, b, preferred_element_type=F32)


def _ln(xt):
    mu = jnp.mean(xt, axis=-1, keepdims=True)
    xc = xt - mu
    var = jnp.mean(xc * xc, axis=-1, keepdims=True)
    return (xc * lax.rsqrt(var + EPS)).astype(BF)


def _ln_chunk(xt, dep=None):
    acc = xt[:, 0:128] if dep is None else xt[:, 0:128] + dep
    for j in range(1, D // 128):
        acc = acc + xt[:, j * 128:(j + 1) * 128]
    mu = jnp.sum(acc, axis=-1, keepdims=True) * (1.0 / D)
    xc = xt - mu
    var = jnp.mean(xc * xc, axis=-1, keepdims=True)
    r = lax.rsqrt(var + EPS)
    return xc * r, r


def _zero_of(v):
    return pltpu.bitcast(pltpu.bitcast(v, U32) & jnp.uint32(0x80000000), F32)


def _phi(t):
    return jnp.where(t > 0, t + 1.0, jnp.exp(t)) + 1e-6


def _recip(d):
    r = pl.reciprocal(d, approx=True)
    return r * (2.0 - d * r)


def _kernel(x_hbm, wa_hbm, woa_hbm, wb_hbm, wob_hbm, out_hbm,
            xin, x, xn_b, xn_0, wq, wo, t_s, k_s, o_s, op_s, z_acc, m_s, zero_s,
            s_buf, m_buf, sem_x0, sem_wa, sem_w, sem_o):

    def x_copy(i):
        r0 = pl.multiple_of(i * XC, XC)
        return pltpu.make_async_copy(x_hbm.at[pl.ds(r0, XC), :], xin.at[pl.ds(r0, XC), :], sem_wa.at[i & 1])

    x0_rows = [(i * 32, 32) for i in range(8)] + [(256 + i * 64, 64) for i in range(4)]
    x0_copies = [pltpu.make_async_copy(x_hbm.at[pl.ds(r, n), :], xin.at[pl.ds(r, n), :], sem_x0.at[i // 8])
                 for i, (r, n) in enumerate(x0_rows)]

    def t_col(j):
        return (1 - (j >> 2)) * (2 * D) + (j & 3) * 256

    def wa_copies(j):
        ct = pl.multiple_of(t_col(j), 256) if not isinstance(j, int) else t_col(j)
        ck = pl.multiple_of(D + j * 128, 128) if not isinstance(j, int) else D + j * 128
        return (pltpu.make_async_copy(wa_hbm.at[:, pl.ds(ct, 256)], wq.at[0, :, pl.ds(ct, 256)], sem_wa.at[j & 1]),
                pltpu.make_async_copy(wa_hbm.at[:, pl.ds(ck, 128)], wq.at[0, :, pl.ds(ck, 128)], sem_wa.at[j & 1]))

    w_copies = [pltpu.make_async_copy(woa_hbm, wo.at[0, :, pl.ds(0, D)], sem_w.at[0]),
                pltpu.make_async_copy(wb_hbm, wq.at[1, :, pl.ds(0, 3 * D)], sem_w.at[0]),
                pltpu.make_async_copy(wob_hbm, wo.at[1, :, pl.ds(0, D)], sem_w.at[0])]

    def out_copy(t):
        return pltpu.make_async_copy(xin.at[pl.ds(t * TM, TM), :], out_hbm.at[pl.ds(t * TM, TM), :], sem_o.at[0])

    def out_copy_last(j):
        r0 = (NTM - 1) * TM + j * 128
        return pltpu.make_async_copy(xin.at[pl.ds(r0, 128), :], out_hbm.at[pl.ds(r0, 128), :], sem_o.at[0])

    def ln_rows(r0, lo, hi, dep=None):
        for c in range(lo, hi, LNC):
            xn, r = _ln_chunk(x[pl.ds(r0 + c, LNC), :], dep)
            xn_b[c // 2:(c + LNC) // 2, :] = _pack(xn)
            if dep is not None:
                dep = _zero_of(r)

    def q_phase(l):
        sel = l & 1
        is_a = sel == 0

        def body(t, carry):
            rt = pl.multiple_of(t * TM, TM)
            rn = pl.multiple_of(jnp.minimum(t + 1, NTM - 1) * TM, TM)
            v = _dot(_unpack(xn_b[0:PRE // 2, :]), wq[sel, :, 2 * D:3 * D])
            t_s[1, :, pl.ds(rt, PRE)] = _pack(v.T)
            CH = (TM - PRE) // G
            for n in range(G):
                c = PRE + n * CH
                dep = None if n < 2 else _zero_of(v[0:CH, (n - 2) * 128:(n - 1) * 128])
                xn, _ = _ln_chunk(x[pl.ds(rt + c, CH), :], dep)
                xn_b[c // 2:(c + CH) // 2, :] = _pack(xn)
            xn_all = _unpack(xn_b[...])
            v = _dot(xn_all[PRE:TM, :], wq[sel, :, 2 * D:3 * D])
            t_s[1, :, pl.ds(rt + PRE, TM - PRE)] = _pack(v.T)
            def tie(qp):
                z = pltpu.bitcast(qp & jnp.uint32(0x80000000), F32)
                return jnp.concatenate(
                    [jnp.concatenate([z[n * 64:(n + 1) * 64, 0:128], z[n * 64:(n + 1) * 64, 128:256],
                                      jnp.zeros((SUB - 128, 128), F32)], axis=0) for n in range(G)], axis=1)

            for sb in range(TM // SUB):
                r0 = pl.multiple_of(t * TM + sb * SUB, SUB)
                xn = xn_all[sb * SUB:(sb + 1) * SUB, :]
                q = _dot(xn, wq[sel, :, 0:D]).T
                qq = jnp.where(is_a, _phi(q), q * QSCALE)
                qp = _pack(qq)
                t_s[0, :, pl.ds(r0, SUB)] = qp
                if sb == 0:
                    dep = _zero_of(qq[0:LNC, 0:128])
            ln_rows(rn, 0, PRE, dep)
            for sb in range(TM // SUB):
                rh = pl.multiple_of(t * (TM // 2) + sb * (SUB // 2), 64)
                k = _dot(xn_all[sb * SUB:(sb + 1) * SUB, :], wq[sel, :, D:2 * D])
                if sb == 0:
                    k = k + tie(qp)
                kk = jnp.where(is_a, _phi(k), k)
                z_acc[...] += jnp.sum(kk.reshape(SUB // 8, 8, D), axis=0)
                kb = _pack(kk)
                for g in range(G):
                    k_s[g, pl.ds(rh, SUB // 2), :] = kb[:, g * 128:(g + 1) * 128]
            return carry

        @pl.when(l > 0)
        def _():
            z_acc[...] = jnp.zeros_like(z_acc)
        lax.fori_loop(jnp.where(l == 0, 1, 0), NTM, body, 0)

    def startup():
        for cp in x0_copies:
            cp.start()
        for cp in wa_copies(0):
            cp.start()
        zero_s[...] = jnp.zeros_like(zero_s)
        for cp in x0_copies[:8]:
            cp.wait()
        xn_0[0:128, :] = _pack(_ln(xin[0:256, :].astype(F32)))
        for cp in x0_copies[8:]:
            cp.wait()
        xn_0[128:256, :] = _pack(_ln(xin[256:512, :].astype(F32)))
        for cp in wa_copies(1):
            cp.start()
        for cp in wa_copies(0):
            cp.wait()

        def body(j, carry):
            xn = _unpack(xn_0[...])
            ct = pl.multiple_of(t_col(j), 256)
            ck = pl.multiple_of(j * 128, 128)
            rc = pl.multiple_of(j * XC, XC)
            xf = xin[pl.ds(rc, XC), :].astype(F32)
            x[pl.ds(rc, XC), :] = xf
            u = pltpu.bitcast(xf, U32)
            u = u[:, 0:512] | u[:, 512:1024]
            u = jnp.concatenate([u[:, 0:256], u[:, 256:512]], axis=0) & jnp.uint32(0x80000000)
            y = (_dot(xn, wq[0, :, pl.ds(ct, 256)]) + pltpu.bitcast(u, F32)).T
            y = jnp.where(j >= 4, _phi(y), y)
            tr = pl.multiple_of((j & 3) * 128, 128)
            t_s[1 - (j >> 2), pl.ds(tr, 128), 0:TM] = _pack(y)
            kk = _phi(_dot(xn, wq[0, :, pl.ds(D + ck, 128)]))
            z_acc[:, pl.ds(ck, 128)] = jnp.sum(kk.reshape(TM // 8, 8, 128), axis=0)
            k_s[j, 0:TM // 2, :] = _pack(kk)
            for c in range(0, PRE, LNC):
                xn1, _ = _ln_chunk(xf[c:c + LNC, :])
                rows = slice(c // 2, (c + LNC) // 2)
                xn_b[rows, :] = jnp.where(j <= TM // XC, _pack(xn1), xn_b[rows, :])

            @pl.when(j + 2 < G)
            def _():
                x_copy(j + 2).start()
                for cp in wa_copies(j + 2):
                    cp.start()

            @pl.when(j == G - 2)
            def _():
                for cp in w_copies:
                    cp.start()

            @pl.when(j + 1 < G)
            def _():
                for cp in wa_copies(j + 1):
                    cp.wait()

                @pl.when(j > 0)
                def _():
                    x_copy(j + 1).wait()
            return carry
        lax.fori_loop(0, G, body, 0)

    def a_mix():
        row = lax.broadcasted_iota(jnp.int32, (128, 128), 0) // DH
        col = lax.broadcasted_iota(jnp.int32, (128, 128), 1) // DH
        same = row == col
        zrow = lax.broadcasted_iota(jnp.int32, (16, 128), 0)
        zcol = lax.broadcasted_iota(jnp.int32, (16, 128), 1) // DH
        zsel = zrow == zcol
        z = jnp.sum(z_acc[...], axis=0, keepdims=True)

        def fold(g, kvg):
            m_s[g * 64:(g + 1) * 64, :] = _pack(_dot(kvg, wo[0, g * 128:(g + 1) * 128, 0:D]))

        def group(g):
            zg = jnp.broadcast_to(z[:, g * 128:(g + 1) * 128], (16, 128))
            zl = jnp.where(zsel, zg, 0.0).astype(BF)
            kvt = None
            for t in range(NTM):
                part = _dot(_unpack(t_s[1, g * 64:(g + 1) * 64, t * TM:(t + 1) * TM]),
                            _unpack(k_s[g, t * TM // 2:(t + 1) * TM // 2, :]))
                kvt = part if kvt is None else kvt + part
                pqt = _unpack(t_s[0, g * 64:(g + 1) * 64, t * TM:(t + 1) * TM])
                r = _recip(_dot(zl, pqt)[0:8, :] + 1e-6)
                pf = pqt.astype(F32)
                ot = jnp.concatenate(
                    [pf[j * DH:(j + 1) * DH, :] * r[j:j + 1, :] for j in range(HPG)], axis=0)
                o_s[g, t * TM // 2:(t + 1) * TM // 2, :] = _pack(ot.T)
            return jnp.where(same, kvt, 0.0).T.astype(BF)

        kvs = []
        for g in range(G):
            kvs.append(group(g))
            if g >= 2:
                fold(g - 2, kvs[g - 2])
        fold(G - 2, kvs[G - 2])
        fold(G - 1, kvs[G - 1])

    def a_out():
        def body(t, carry):
            for sb in range(TM // SUB):
                r0 = pl.multiple_of(t * TM + sb * SUB, SUB)
                rh = pl.multiple_of(t * (TM // 2) + sb * (SUB // 2), SUB // 2)
                o = jnp.concatenate([_unpack(o_s[g, pl.ds(rh, SUB // 2), :]) for g in range(G)], axis=1)
                xnew = x[pl.ds(r0, SUB), :] + _dot(o, _unpack(m_s[...]))
                x[pl.ds(r0, SUB), :] = xnew
                if sb == 0:
                    for c in range(0, PRE, LNC):
                        xn, _ = _ln_chunk(xnew[c:c + LNC, :])
                        rows = slice(c // 2, (c + LNC) // 2)
                        xn_b[rows, :] = jnp.where(t == 0, _pack(xn), xn_b[rows, :])
            return carry
        lax.fori_loop(0, NTM, body, 0)

    def decode(b):
        return b & (G - 1), b >> 3

    def get_qm(b, hh):
        g, qi = decode(b)
        qoff = pl.multiple_of(qi * TQ, TQ)
        if isinstance(hh, int):
            roff = pl.multiple_of(g * 64 + hh * 16, 16)
            parts = []
            if hh > 0:
                parts.append(jnp.zeros((hh * 16, TQ), U32))
            parts.append(t_s[0, pl.ds(roff, 16), pl.ds(qoff, TQ)])
            if hh < HPG - 1:
                parts.append(jnp.zeros(((HPG - 1 - hh) * 16, TQ), U32))
            return _unpack(jnp.concatenate(parts, axis=0))
        roff = pl.multiple_of(g * 64, 64)
        qg = t_s[0, pl.ds(roff, 64), pl.ds(qoff, TQ)]
        row = lax.broadcasted_iota(jnp.int32, (64, TQ), 0) // 16
        return _unpack(jnp.where(row == hh, qg, jnp.zeros_like(qg)))

    def qk_chunk(g, qm, c, hh, m8):
        kc = _unpack(k_s[g, c * TK // 2:(c + 1) * TK // 2, :])
        s = _dot(kc, qm)
        s_buf[hh, c * TK:(c + 1) * TK, :] = s
        mc = jnp.max(s.reshape(TK // 8, 8, TQ), axis=0)
        return mc if m8 is None else jnp.maximum(m8, mc)

    def out_proj(b, o):
        g, qi = decode(b)
        r0 = pl.multiple_of(qi * TQ, TQ)
        w0 = pl.multiple_of(g * 128, 128)
        xnew = x[pl.ds(r0, TQ), :] + _dot(o, wo[1, pl.ds(w0, 128), 0:D])
        x[pl.ds(r0, TQ), :] = xnew
        xin[pl.ds(r0, TQ), :] = xnew.astype(BF)

    def lsum(p, l8):
        for r in range(TK // 16 - 1, -1, -1):
            pr = p[r * 16:r * 16 + 8, :] + p[r * 16 + 8:r * 16 + 16, :]
            l8 = pr if l8 is None else l8 + pr
        return l8

    def attn_block(b):
        gc, _ = decode(b)
        gn = (b + 1) & (G - 1)
        o_prev = _unpack(op_s[...])
        outs = []
        ms = [m_buf[hh] for hh in range(HPG)]
        for hh in range(HPG):
            qm = get_qm(b + 1, hh)
            voff = pl.multiple_of(gc * 64 + hh * 16, 16)
            l8 = None
            o = zero_s[...]
            m8 = None
            for c in range(NK):
                p = jnp.exp2(s_buf[hh, c * TK:(c + 1) * TK, :] - ms[hh])
                l8 = lsum(p, l8)
                m8 = qk_chunk(gn, qm, c, hh, m8)
                vc = _unpack(t_s[1, pl.ds(voff, 16), c * TK:(c + 1) * TK])
                o = o + _dot(vc, p.astype(BF))
            m_buf[hh] = jnp.max(m8, axis=0, keepdims=True)
            l = jnp.sum(l8, axis=0, keepdims=True)
            outs.append(o * _recip(l))
        out_proj(jnp.maximum(b - 1, 0), o_prev)
        ot = jnp.concatenate(outs, axis=0)
        op_s[...] = _pack(ot.T)

    def attn_last(is_last_layer):
        rbase = (NQ - 1) * TQ

        def proj_piece(o, g, r, cc, final):
            r0 = rbase + r
            cols = slice(cc * 256, (cc + 1) * 256)
            xnew = x[r0:r0 + 128, cols] + _dot(o, wo[1, g * 128:(g + 1) * 128, cols])
            x[r0:r0 + 128, cols] = xnew
            if final:
                xin[r0:r0 + 128, cols] = xnew.astype(BF)
                if cc == 3:
                    @pl.when(is_last_layer)
                    def _():
                        out_copy_last(r // 128).start()

        o_prev = _unpack(op_s[...])
        queue = [(o_prev[r:r + 128, :], G - 2, r, cc, False) for r in range(0, TQ, 128) for cc in range(4)]
        work = 0
        for q0, q1, ek in ((0, 256, 256), (256, 384, 512), (384, 512, 512)):
            cols = slice(q0, q1)
            outs = []
            for hh in range(HPG):
                m = m_buf[hh, :, cols]
                voff = (G - 1) * 64 + hh * 16
                l8 = None
                o = zero_s[:, 0:q1 - q0]
                for c in range(S // ek):
                    p = jnp.exp2(s_buf[hh, c * ek:(c + 1) * ek, cols] - m)
                    for u in range(ek // TK):
                        l8 = lsum(p[u * TK:(u + 1) * TK, :], l8)
                    vc = _unpack(t_s[1, voff:voff + 16, c * ek:(c + 1) * ek])
                    o = o + _dot(vc, p.astype(BF))
                    work += ek * (q1 - q0) // 1024
                    while queue and work >= 128:
                        work -= 128
                        proj_piece(*queue.pop(0))
                    if not queue:
                        work = 0
                l = jnp.sum(l8, axis=0, keepdims=True)
                outs.append(o * _recip(l))
            oj = jnp.concatenate(outs, axis=0).T.astype(BF)
            if not queue:
                work = -192
            queue += [(oj[r:r + 128, :], G - 1, q0 + r, cc, True) for r in range(0, q1 - q0, 128) for cc in range(4)]
        while queue:
            proj_piece(*queue.pop(0))

    def attention(is_last_layer):
        op_s[...] = jnp.zeros_like(op_s)

        def pro(i, carry):
            for u in range(2):
                hh = 2 * i + u
                qm = get_qm(0, hh)
                m8 = None
                for c in range(NK):
                    m8 = qk_chunk(0, qm, c, hh, m8)
                m_buf[hh] = jnp.max(m8, axis=0, keepdims=True)
            return carry
        lax.fori_loop(0, HPG // 2, pro, 0)

        def body(b, carry):
            @pl.when(jnp.logical_and(is_last_layer, jnp.logical_and((b & (G - 1)) == 1, b > G)))
            def _():
                out_copy((b >> 3) - 1).start()
            attn_block(b)
            return carry
        lax.fori_loop(0, NBLK - 1, body, 0)
        ln_rows(0, 0, PRE)
        attn_last(is_last_layer)

    startup()

    def layer(l, carry):
        sel = l & 1
        q_phase(l)

        @pl.when(l == 0)
        def _():
            for cp in w_copies:
                cp.wait()

        @pl.when(sel == 0)
        def _():
            a_mix()
            a_out()

        @pl.when(sel == 1)
        def _():
            attention(l == 3)
        return carry

    lax.fori_loop(0, 4, layer, 0)
    for t in range(NTM - 1):
        out_copy(t).wait()
    for j in range(TM // 128):
        out_copy_last(j).wait()


@jax.jit
def pallas_interleave_layers__linear_attn_block__mha_block__prompt_kernel(A_x, A_wqkv, A_wo, B_x, B_wqkv, B_wo):
    del B_x
    scratch = [
        pltpu.VMEM((S, D), BF),
        pltpu.VMEM((S, D), F32),
        pltpu.VMEM((TM // 2, D), U32),
        pltpu.VMEM((TM // 2, D), U32),
        pltpu.VMEM((2, D, 3 * D + WPAD), BF),
        pltpu.VMEM((2, D, D + WPAD), BF),
        pltpu.VMEM((2, D // 2, S), U32),
        pltpu.VMEM((G, S // 2, 128), U32),
        pltpu.VMEM((G, S // 2, 128), U32),
        pltpu.VMEM((TQ // 2, 128), U32),
        pltpu.VMEM((8, D), F32),
        pltpu.VMEM((D // 2, D), U32),
        pltpu.VMEM((DH, TQ), F32),
        pltpu.VMEM((HPG, S, TQ), F32),
        pltpu.VMEM((HPG, 1, TQ), F32),
        pltpu.SemaphoreType.DMA((2,)),
        pltpu.SemaphoreType.DMA((2,)),
        pltpu.SemaphoreType.DMA((1,)),
        pltpu.SemaphoreType.DMA((1,)),
    ]
    out = pl.pallas_call(
        _kernel,
        out_shape=jax.ShapeDtypeStruct((S, D), BF),
        in_specs=[pl.BlockSpec(memory_space=pl.ANY)] * 5,
        out_specs=pl.BlockSpec(memory_space=pl.ANY),
        scratch_shapes=scratch,
        compiler_params=pltpu.CompilerParams(
            vmem_limit_bytes=120 * 1024 * 1024,
            disable_bounds_checks=True,
            disable_semaphore_checks=True,
        ),
    )(A_x.reshape(S, D), A_wqkv, A_wo, B_wqkv, B_wo)
    return out.reshape(1, S, D)
```

```python
import math

import jax
import jax.numpy as jnp
from jax import lax
import jax.experimental.pallas as pl
import jax.experimental.pallas.tpu as pltpu

S, D, H, DH = 2048, 1024, 32, 32
G = D // 128
HPG = 128 // DH
TM = 512
NTM = S // TM
SUB = 256
TQ = 512
TK = 128
NQ = S // TQ
NK = S // TK
NBLK = G * NQ
PRE = 128
LNC = 32
XC = S // G
EPS = 1e-5
WPAD = 256
QSCALE = (DH ** -0.5) * math.log2(math.e)
BF = jnp.bfloat16
F32 = jnp.float32
U32 = jnp.uint32


def _pack(v):
    return pltpu.bitcast(v.astype(BF), U32)


def _unpack(u):
    return pltpu.bitcast(u, BF)


def _dot(a, b):
    return jnp.dot(a, b, preferred_element_type=F32)


def _ln(xt):
    mu = jnp.mean(xt, axis=-1, keepdims=True)
    xc = xt - mu
    var = jnp.mean(xc * xc, axis=-1, keepdims=True)
    return (xc * lax.rsqrt(var + EPS)).astype(BF)


def _ln_chunk(xt, dep=None):
    acc = xt[:, 0:128] if dep is None else xt[:, 0:128] + dep
    for j in range(1, D // 128):
        acc = acc + xt[:, j * 128:(j + 1) * 128]
    mu = jnp.sum(acc, axis=-1, keepdims=True) * (1.0 / D)
    xc = xt - mu
    var = jnp.mean(xc * xc, axis=-1, keepdims=True)
    r = lax.rsqrt(var + EPS)
    return xc * r, r


def _zero_of(v):
    return pltpu.bitcast(pltpu.bitcast(v, U32) & jnp.uint32(0x80000000), F32)


def _tie(qp):
    z = pltpu.bitcast(qp & jnp.uint32(0x80000000), F32)
    return jnp.concatenate(
        [jnp.concatenate([z[n * 64:(n + 1) * 64, 0:128], z[n * 64:(n + 1) * 64, 128:256],
                          jnp.zeros((SUB - 128, 128), F32)], axis=0) for n in range(G)], axis=1)


def _phi(t):
    return jnp.where(t > 0, t + 1.0, jnp.exp(t)) + 1e-6


def _recip(d):
    r = pl.reciprocal(d, approx=True)
    return r * (2.0 - d * r)


def _kernel(x_hbm, wa_hbm, woa_hbm, wb_hbm, wob_hbm, out_hbm,
            xin, x, xn_b, xn_0, wq, wo, t_s, k_s, o_s, op_s, z_acc, m_s, zero_s,
            s_buf, m_buf, sem_x0, sem_wa, sem_w, sem_o):

    def x_copy(i):
        r0 = pl.multiple_of(i * XC, XC)
        return pltpu.make_async_copy(x_hbm.at[pl.ds(r0, XC), :], xin.at[pl.ds(r0, XC), :], sem_wa.at[i & 1])

    x0_rows = [(i * 32, 32) for i in range(8)] + [(256 + i * 64, 64) for i in range(4)]
    x0_copies = [pltpu.make_async_copy(x_hbm.at[pl.ds(r, n), :], xin.at[pl.ds(r, n), :], sem_x0.at[i // 8])
                 for i, (r, n) in enumerate(x0_rows)]

    def t_col(j):
        return (1 - (j >> 2)) * (2 * D) + (j & 3) * 256

    def wa_copies(j):
        ct = pl.multiple_of(t_col(j), 256) if not isinstance(j, int) else t_col(j)
        ck = pl.multiple_of(D + j * 128, 128) if not isinstance(j, int) else D + j * 128
        return (pltpu.make_async_copy(wa_hbm.at[:, pl.ds(ct, 256)], wq.at[0, :, pl.ds(ct, 256)], sem_wa.at[j & 1]),
                pltpu.make_async_copy(wa_hbm.at[:, pl.ds(ck, 128)], wq.at[0, :, pl.ds(ck, 128)], sem_wa.at[j & 1]))

    w_copies = [pltpu.make_async_copy(woa_hbm, wo.at[0, :, pl.ds(0, D)], sem_w.at[0]),
                pltpu.make_async_copy(wb_hbm, wq.at[1, :, pl.ds(0, 3 * D)], sem_w.at[0]),
                pltpu.make_async_copy(wob_hbm, wo.at[1, :, pl.ds(0, D)], sem_w.at[0])]

    def out_copy(t):
        return pltpu.make_async_copy(xin.at[pl.ds(t * TM, TM), :], out_hbm.at[pl.ds(t * TM, TM), :], sem_o.at[0])

    def out_copy_last(j):
        r0 = (NTM - 1) * TM + j * 128
        return pltpu.make_async_copy(xin.at[pl.ds(r0, 128), :], out_hbm.at[pl.ds(r0, 128), :], sem_o.at[0])

    def ln_rows(r0, lo, hi, dep=None):
        for c in range(lo, hi, LNC):
            xn, r = _ln_chunk(x[pl.ds(r0 + c, LNC), :], dep)
            xn_b[c // 2:(c + LNC) // 2, :] = _pack(xn)
            if dep is not None:
                dep = _zero_of(r)

    def q_phase(l):
        sel = l & 1
        is_a = sel == 0

        def body(t, carry):
            rt = pl.multiple_of(t * TM, TM)
            rn = pl.multiple_of(jnp.minimum(t + 1, NTM - 1) * TM, TM)
            v = _dot(_unpack(xn_b[0:PRE // 2, :]), wq[sel, :, 2 * D:3 * D])
            t_s[1, :, pl.ds(rt, PRE)] = _pack(v.T)
            CH = (TM - PRE) // G
            for n in range(G):
                c = PRE + n * CH
                dep = None if n < 2 else _zero_of(v[0:CH, (n - 2) * 128:(n - 1) * 128])
                xn, _ = _ln_chunk(x[pl.ds(rt + c, CH), :], dep)
                xn_b[c // 2:(c + CH) // 2, :] = _pack(xn)
            xn_all = _unpack(xn_b[...])
            v = _dot(xn_all[PRE:TM, :], wq[sel, :, 2 * D:3 * D])
            t_s[1, :, pl.ds(rt + PRE, TM - PRE)] = _pack(v.T)
            for sb in range(TM // SUB):
                r0 = pl.multiple_of(t * TM + sb * SUB, SUB)
                xn = xn_all[sb * SUB:(sb + 1) * SUB, :]
                q = _dot(xn, wq[sel, :, 0:D]).T
                qq = jnp.where(is_a, _phi(q), q * QSCALE)
                qp = _pack(qq)
                t_s[0, :, pl.ds(r0, SUB)] = qp
                if sb == 0:
                    dep = _zero_of(qq[0:LNC, 0:128])
            ln_rows(rn, 0, PRE, dep)
            for sb in range(TM // SUB):
                rh = pl.multiple_of(t * (TM // 2) + sb * (SUB // 2), 64)
                k = _dot(xn_all[sb * SUB:(sb + 1) * SUB, :], wq[sel, :, D:2 * D])
                if sb == 0:
                    k = k + _tie(qp)
                kk = jnp.where(is_a, _phi(k), k)
                z_acc[...] += jnp.sum(kk.reshape(SUB // 8, 8, D), axis=0)
                kb = _pack(kk)
                for g in range(G):
                    k_s[g, pl.ds(rh, SUB // 2), :] = kb[:, g * 128:(g + 1) * 128]
            return carry

        @pl.when(l > 0)
        def _():
            z_acc[...] = jnp.zeros_like(z_acc)
        lax.fori_loop(jnp.where(l == 0, 1, 0), NTM, body, 0)

    def startup():
        for cp in x0_copies:
            cp.start()
        for cp in wa_copies(0):
            cp.start()
        zero_s[...] = jnp.zeros_like(zero_s)
        for cp in x0_copies[:8]:
            cp.wait()
        xn_0[0:128, :] = _pack(_ln(xin[0:256, :].astype(F32)))
        for cp in x0_copies[8:]:
            cp.wait()
        xn_0[128:256, :] = _pack(_ln(xin[256:512, :].astype(F32)))
        for cp in wa_copies(1):
            cp.start()
        for cp in wa_copies(0):
            cp.wait()

        def body(j, carry):
            xn = _unpack(xn_0[...])
            ct = pl.multiple_of(t_col(j), 256)
            ck = pl.multiple_of(j * 128, 128)
            rc = pl.multiple_of(j * XC, XC)
            xf = xin[pl.ds(rc, XC), :].astype(F32)
            x[pl.ds(rc, XC), :] = xf
            u = pltpu.bitcast(xf, U32)
            u = u[:, 0:512] | u[:, 512:1024]
            u = jnp.concatenate([u[:, 0:256], u[:, 256:512]], axis=0) & jnp.uint32(0x80000000)
            y = (_dot(xn, wq[0, :, pl.ds(ct, 256)]) + pltpu.bitcast(u, F32)).T
            y = jnp.where(j >= 4, _phi(y), y)
            tr = pl.multiple_of((j & 3) * 128, 128)
            t_s[1 - (j >> 2), pl.ds(tr, 128), 0:TM] = _pack(y)
            kk = _phi(_dot(xn, wq[0, :, pl.ds(D + ck, 128)]))
            z_acc[:, pl.ds(ck, 128)] = jnp.sum(kk.reshape(TM // 8, 8, 128), axis=0)
            k_s[j, 0:TM // 2, :] = _pack(kk)
            for c in range(0, PRE, LNC):
                xn1, _ = _ln_chunk(xf[c:c + LNC, :])
                rows = slice(c // 2, (c + LNC) // 2)
                xn_b[rows, :] = jnp.where(j <= TM // XC, _pack(xn1), xn_b[rows, :])

            @pl.when(j + 2 < G)
            def _():
                x_copy(j + 2).start()
                for cp in wa_copies(j + 2):
                    cp.start()

            @pl.when(j == G - 2)
            def _():
                for cp in w_copies:
                    cp.start()

            @pl.when(j + 1 < G)
            def _():
                for cp in wa_copies(j + 1):
                    cp.wait()

                @pl.when(j > 0)
                def _():
                    x_copy(j + 1).wait()
            return carry
        lax.fori_loop(0, G, body, 0)

    def a_mix():
        row = lax.broadcasted_iota(jnp.int32, (128, 128), 0) // DH
        col = lax.broadcasted_iota(jnp.int32, (128, 128), 1) // DH
        same = row == col
        zrow = lax.broadcasted_iota(jnp.int32, (16, 128), 0)
        zcol = lax.broadcasted_iota(jnp.int32, (16, 128), 1) // DH
        zsel = zrow == zcol
        z = jnp.sum(z_acc[...], axis=0, keepdims=True)

        def fold(g, kvg):
            m_s[g * 64:(g + 1) * 64, :] = _pack(_dot(kvg, wo[0, g * 128:(g + 1) * 128, 0:D]))

        def group(g):
            zg = jnp.broadcast_to(z[:, g * 128:(g + 1) * 128], (16, 128))
            zl = jnp.where(zsel, zg, 0.0).astype(BF)
            kvt = None
            for t in range(NTM):
                part = _dot(_unpack(t_s[1, g * 64:(g + 1) * 64, t * TM:(t + 1) * TM]),
                            _unpack(k_s[g, t * TM // 2:(t + 1) * TM // 2, :]))
                kvt = part if kvt is None else kvt + part
                pqt = _unpack(t_s[0, g * 64:(g + 1) * 64, t * TM:(t + 1) * TM])
                r = _recip(_dot(zl, pqt)[0:8, :] + 1e-6)
                pf = pqt.astype(F32)
                ot = jnp.concatenate(
                    [pf[j * DH:(j + 1) * DH, :] * r[j:j + 1, :] for j in range(HPG)], axis=0)
                o_s[g, t * TM // 2:(t + 1) * TM // 2, :] = _pack(ot.T)
            return jnp.where(same, kvt, 0.0).T.astype(BF)

        kvs = []
        for g in range(G):
            kvs.append(group(g))
            if g >= 2:
                fold(g - 2, kvs[g - 2])
        fold(G - 2, kvs[G - 2])
        fold(G - 1, kvs[G - 1])

    def a_out():
        def body(t, carry):
            for sb in range(TM // SUB):
                r0 = pl.multiple_of(t * TM + sb * SUB, SUB)
                rh = pl.multiple_of(t * (TM // 2) + sb * (SUB // 2), SUB // 2)
                o = jnp.concatenate([_unpack(o_s[g, pl.ds(rh, SUB // 2), :]) for g in range(G)], axis=1)
                xnew = x[pl.ds(r0, SUB), :] + _dot(o, _unpack(m_s[...]))
                x[pl.ds(r0, SUB), :] = xnew
                if sb == 0:
                    for c in range(0, PRE, LNC):
                        xn, _ = _ln_chunk(xnew[c:c + LNC, :])
                        rows = slice(c // 2, (c + LNC) // 2)
                        xn_b[rows, :] = jnp.where(t == 0, _pack(xn), xn_b[rows, :])
            return carry
        lax.fori_loop(0, NTM, body, 0)

    def decode(b):
        return b & (G - 1), b >> 3

    def get_qm(b, hh):
        g, qi = decode(b)
        qoff = pl.multiple_of(qi * TQ, TQ)
        if isinstance(hh, int):
            roff = pl.multiple_of(g * 64 + hh * 16, 16)
            parts = []
            if hh > 0:
                parts.append(jnp.zeros((hh * 16, TQ), U32))
            parts.append(t_s[0, pl.ds(roff, 16), pl.ds(qoff, TQ)])
            if hh < HPG - 1:
                parts.append(jnp.zeros(((HPG - 1 - hh) * 16, TQ), U32))
            return _unpack(jnp.concatenate(parts, axis=0))
        roff = pl.multiple_of(g * 64, 64)
        qg = t_s[0, pl.ds(roff, 64), pl.ds(qoff, TQ)]
        row = lax.broadcasted_iota(jnp.int32, (64, TQ), 0) // 16
        return _unpack(jnp.where(row == hh, qg, jnp.zeros_like(qg)))

    def qk_chunk(g, qm, c, hh, m8):
        kc = _unpack(k_s[g, c * TK // 2:(c + 1) * TK // 2, :])
        s = _dot(kc, qm)
        s_buf[hh, c * TK:(c + 1) * TK, :] = s
        mc = jnp.max(s.reshape(TK // 8, 8, TQ), axis=0)
        return mc if m8 is None else jnp.maximum(m8, mc)

    def out_proj(b, o):
        g, qi = decode(b)
        r0 = pl.multiple_of(qi * TQ, TQ)
        w0 = pl.multiple_of(g * 128, 128)
        xnew = x[pl.ds(r0, TQ), :] + _dot(o, wo[1, pl.ds(w0, 128), 0:D])
        x[pl.ds(r0, TQ), :] = xnew
        xin[pl.ds(r0, TQ), :] = xnew.astype(BF)

    def lsum(p, l8):
        for r in range(TK // 16 - 1, -1, -1):
            pr = p[r * 16:r * 16 + 8, :] + p[r * 16 + 8:r * 16 + 16, :]
            l8 = pr if l8 is None else l8 + pr
        return l8

    def attn_block(b):
        gc, _ = decode(b)
        gn = (b + 1) & (G - 1)
        o_prev = _unpack(op_s[...])
        outs = []
        ms = [m_buf[hh] for hh in range(HPG)]
        for hh in range(HPG):
            qm = get_qm(b + 1, hh)
            voff = pl.multiple_of(gc * 64 + hh * 16, 16)
            l8 = None
            o = zero_s[...]
            m8 = None
            for c in range(NK):
                p = jnp.exp2(s_buf[hh, c * TK:(c + 1) * TK, :] - ms[hh])
                l8 = lsum(p, l8)
                m8 = qk_chunk(gn, qm, c, hh, m8)
                vc = _unpack(t_s[1, pl.ds(voff, 16), c * TK:(c + 1) * TK])
                o = o + _dot(vc, p.astype(BF))
            m_buf[hh] = jnp.max(m8, axis=0, keepdims=True)
            l = jnp.sum(l8, axis=0, keepdims=True)
            outs.append(o * _recip(l))
        out_proj(jnp.maximum(b - 1, 0), o_prev)
        ot = jnp.concatenate(outs, axis=0)
        op_s[...] = _pack(ot.T)

    def attn_last(is_last_layer):
        rbase = (NQ - 1) * TQ

        def proj_piece(o, g, r, cc, final):
            r0 = rbase + r
            cols = slice(cc * 256, (cc + 1) * 256)
            xnew = x[r0:r0 + 128, cols] + _dot(o, wo[1, g * 128:(g + 1) * 128, cols])
            x[r0:r0 + 128, cols] = xnew
            if final:
                xin[r0:r0 + 128, cols] = xnew.astype(BF)
                if cc == 3:
                    @pl.when(is_last_layer)
                    def _():
                        out_copy_last(r // 128).start()

        o_prev = _unpack(op_s[...])
        queue = [(o_prev[r:r + 128, :], G - 2, r, cc, False) for r in range(0, TQ, 128) for cc in range(4)]
        work = 0
        for q0, q1, ek in ((0, 256, 256), (256, 384, 512), (384, 512, 512)):
            cols = slice(q0, q1)
            outs = []
            for hh in range(HPG):
                m = m_buf[hh, :, cols]
                voff = (G - 1) * 64 + hh * 16
                l8 = None
                o = zero_s[:, 0:q1 - q0]
                for c in range(S // ek):
                    p = jnp.exp2(s_buf[hh, c * ek:(c + 1) * ek, cols] - m)
                    for u in range(ek // TK):
                        l8 = lsum(p[u * TK:(u + 1) * TK, :], l8)
                    vc = _unpack(t_s[1, voff:voff + 16, c * ek:(c + 1) * ek])
                    o = o + _dot(vc, p.astype(BF))
                    work += ek * (q1 - q0) // 1024
                    while queue and work >= 128:
                        work -= 128
                        proj_piece(*queue.pop(0))
                    if not queue:
                        work = 0
                l = jnp.sum(l8, axis=0, keepdims=True)
                outs.append(o * _recip(l))
            oj = jnp.concatenate(outs, axis=0).T.astype(BF)
            if not queue:
                work = -192
            queue += [(oj[r:r + 128, :], G - 1, q0 + r, cc, True) for r in range(0, q1 - q0, 128) for cc in range(4)]
        while queue:
            proj_piece(*queue.pop(0))

    def attention(is_last_layer):
        op_s[...] = jnp.zeros_like(op_s)

        def pro(i, carry):
            for u in range(2):
                hh = 2 * i + u
                qm = get_qm(0, hh)
                m8 = None
                for c in range(NK):
                    m8 = qk_chunk(0, qm, c, hh, m8)
                m_buf[hh] = jnp.max(m8, axis=0, keepdims=True)
            return carry
        lax.fori_loop(0, HPG // 2, pro, 0)

        def body(b, carry):
            @pl.when(jnp.logical_and(is_last_layer, jnp.logical_and((b & (G - 1)) == 1, b > G)))
            def _():
                out_copy((b >> 3) - 1).start()
            attn_block(b)
            return carry
        lax.fori_loop(0, NBLK - 1, body, 0)
        ln_rows(0, 0, PRE)
        attn_last(is_last_layer)

    startup()

    def layer(l, carry):
        sel = l & 1
        q_phase(l)

        @pl.when(l == 0)
        def _():
            for cp in w_copies:
                cp.wait()

        @pl.when(sel == 0)
        def _():
            a_mix()
            a_out()

        @pl.when(sel == 1)
        def _():
            attention(l == 3)
        return carry

    lax.fori_loop(0, 4, layer, 0)
    for t in range(NTM - 1):
        out_copy(t).wait()
    for j in range(TM // 128):
        out_copy_last(j).wait()


@jax.jit
def pallas_interleave_layers__linear_attn_block__mha_block__prompt_kernel(A_x, A_wqkv, A_wo, B_x, B_wqkv, B_wo):
    del B_x
    scratch = [
        pltpu.VMEM((S, D), BF),
        pltpu.VMEM((S, D), F32),
        pltpu.VMEM((TM // 2, D), U32),
        pltpu.VMEM((TM // 2, D), U32),
        pltpu.VMEM((2, D, 3 * D + WPAD), BF),
        pltpu.VMEM((2, D, D + WPAD), BF),
        pltpu.VMEM((2, D // 2, S), U32),
        pltpu.VMEM((G, S // 2, 128), U32),
        pltpu.VMEM((G, S // 2, 128), U32),
        pltpu.VMEM((TQ // 2, 128), U32),
        pltpu.VMEM((8, D), F32),
        pltpu.VMEM((D // 2, D), U32),
        pltpu.VMEM((DH, TQ), F32),
        pltpu.VMEM((HPG, S, TQ), F32),
        pltpu.VMEM((HPG, 1, TQ), F32),
        pltpu.SemaphoreType.DMA((2,)),
        pltpu.SemaphoreType.DMA((2,)),
        pltpu.SemaphoreType.DMA((1,)),
        pltpu.SemaphoreType.DMA((1,)),
    ]
    out = pl.pallas_call(
        _kernel,
        out_shape=jax.ShapeDtypeStruct((S, D), BF),
        in_specs=[pl.BlockSpec(memory_space=pl.ANY)] * 5,
        out_specs=pl.BlockSpec(memory_space=pl.ANY),
        scratch_shapes=scratch,
        compiler_params=pltpu.CompilerParams(
            vmem_limit_bytes=120 * 1024 * 1024,
            disable_bounds_checks=True,
            disable_semaphore_checks=True,
        ),
    )(A_x.reshape(S, D), A_wqkv, A_wo, B_wqkv, B_wo)
    return out.reshape(1, S, D)
```

```python
import math

import jax
import jax.numpy as jnp
from jax import lax
import jax.experimental.pallas as pl
import jax.experimental.pallas.tpu as pltpu

S, D, H, DH = 2048, 1024, 32, 32
G = D // 128
HPG = 128 // DH
TM = 512
NTM = S // TM
SUB = 256
TQ = 512
TK = 128
NQ = S // TQ
NK = S // TK
NBLK = G * NQ
PRE = 128
LNC = 32
XC = S // G
EPS = 1e-5
WPAD = 256
QSCALE = (DH ** -0.5) * math.log2(math.e)
BF = jnp.bfloat16
F32 = jnp.float32
U32 = jnp.uint32


def _pack(v):
    return pltpu.bitcast(v.astype(BF), U32)


def _unpack(u):
    return pltpu.bitcast(u, BF)


def _dot(a, b):
    return jnp.dot(a, b, preferred_element_type=F32)


def _ln(xt):
    mu = jnp.mean(xt, axis=-1, keepdims=True)
    xc = xt - mu
    var = jnp.mean(xc * xc, axis=-1, keepdims=True)
    return (xc * lax.rsqrt(var + EPS)).astype(BF)


def _ln_chunk(xt, dep=None):
    acc = xt[:, 0:128] if dep is None else xt[:, 0:128] + dep
    for j in range(1, D // 128):
        acc = acc + xt[:, j * 128:(j + 1) * 128]
    mu = jnp.sum(acc, axis=-1, keepdims=True) * (1.0 / D)
    xc = xt - mu
    var = jnp.mean(xc * xc, axis=-1, keepdims=True)
    r = lax.rsqrt(var + EPS)
    return xc * r, r


def _zero_of(v):
    return pltpu.bitcast(pltpu.bitcast(v, U32) & jnp.uint32(0x80000000), F32)


def _tie(qp):
    z = pltpu.bitcast(qp & jnp.uint32(0x80000000), F32)
    return jnp.concatenate(
        [jnp.concatenate([z[n * 64:(n + 1) * 64, 0:128], z[n * 64:(n + 1) * 64, 128:256],
                          jnp.zeros((SUB - 128, 128), F32)], axis=0) for n in range(G)], axis=1)


def _phi(t):
    return jnp.where(t > 0, t + 1.0, jnp.exp(t)) + 1e-6


def _recip(d):
    r = pl.reciprocal(d, approx=True)
    return r * (2.0 - d * r)


def _kernel(x_hbm, wa_hbm, woa_hbm, wb_hbm, wob_hbm, out_hbm,
            xin, x, xn_b, xn_0, wq, wo, t_s, k_s, o_s, op_s, z_acc, m_s, zero_s,
            s_buf, m_buf, sem_x0, sem_wa, sem_w, sem_o):

    def x_copy(i):
        r0 = pl.multiple_of(i * XC, XC)
        return pltpu.make_async_copy(x_hbm.at[pl.ds(r0, XC), :], xin.at[pl.ds(r0, XC), :], sem_wa.at[i & 1])

    x0_rows = [(i * 32, 32) for i in range(8)] + [(256 + i * 64, 64) for i in range(4)]
    x0_copies = [pltpu.make_async_copy(x_hbm.at[pl.ds(r, n), :], xin.at[pl.ds(r, n), :], sem_x0.at[i // 8])
                 for i, (r, n) in enumerate(x0_rows)]

    def t_col(j):
        return (1 - (j >> 2)) * (2 * D) + (j & 3) * 256

    def wa_copies(j):
        ct = pl.multiple_of(t_col(j), 256) if not isinstance(j, int) else t_col(j)
        ck = pl.multiple_of(D + j * 128, 128) if not isinstance(j, int) else D + j * 128
        return (pltpu.make_async_copy(wa_hbm.at[:, pl.ds(ct, 256)], wq.at[0, :, pl.ds(ct, 256)], sem_wa.at[j & 1]),
                pltpu.make_async_copy(wa_hbm.at[:, pl.ds(ck, 128)], wq.at[0, :, pl.ds(ck, 128)], sem_wa.at[j & 1]))

    w_copies = [pltpu.make_async_copy(woa_hbm, wo.at[0, :, pl.ds(0, D)], sem_w.at[0]),
                pltpu.make_async_copy(wb_hbm, wq.at[1, :, pl.ds(0, 3 * D)], sem_w.at[0]),
                pltpu.make_async_copy(wob_hbm, wo.at[1, :, pl.ds(0, D)], sem_w.at[0])]

    def out_copy(t):
        return pltpu.make_async_copy(xin.at[pl.ds(t * TM, TM), :], out_hbm.at[pl.ds(t * TM, TM), :], sem_o.at[0])

    def out_copy_last(j):
        r0 = (NTM - 1) * TM + j * 128
        return pltpu.make_async_copy(xin.at[pl.ds(r0, 128), :], out_hbm.at[pl.ds(r0, 128), :], sem_o.at[0])

    def ln_rows(r0, lo, hi, dep=None):
        for c in range(lo, hi, LNC):
            xn, r = _ln_chunk(x[pl.ds(r0 + c, LNC), :], dep)
            xn_b[c // 2:(c + LNC) // 2, :] = _pack(xn)
            if dep is not None:
                dep = _zero_of(r)

    def q_phase(l):
        sel = l & 1
        is_a = sel == 0

        def body(t, carry):
            rt = pl.multiple_of(t * TM, TM)
            rn = pl.multiple_of(jnp.minimum(t + 1, NTM - 1) * TM, TM)
            v = _dot(_unpack(xn_b[0:PRE // 2, :]), wq[sel, :, 2 * D:3 * D])
            t_s[1, :, pl.ds(rt, PRE)] = _pack(v.T)
            CH = (TM - PRE) // G
            for n in range(G):
                c = PRE + n * CH
                dep = None if n < 2 else _zero_of(v[0:CH, (n - 2) * 128:(n - 1) * 128])
                xn, _ = _ln_chunk(x[pl.ds(rt + c, CH), :], dep)
                xn_b[c // 2:(c + CH) // 2, :] = _pack(xn)
            xn_all = _unpack(xn_b[...])
            v = _dot(xn_all[PRE:TM, :], wq[sel, :, 2 * D:3 * D])
            t_s[1, :, pl.ds(rt + PRE, TM - PRE)] = _pack(v.T)
            for sb in range(TM // SUB):
                r0 = pl.multiple_of(t * TM + sb * SUB, SUB)
                xn = xn_all[sb * SUB:(sb + 1) * SUB, :]
                q = _dot(xn, wq[sel, :, 0:D]).T
                qq = jnp.where(is_a, _phi(q), q * QSCALE)
                qp = _pack(qq)
                t_s[0, :, pl.ds(r0, SUB)] = qp
                if sb == 0:
                    dep = _zero_of(qq[0:LNC, 0:128])
            ln_rows(rn, 0, PRE, dep)
            for sb in range(TM // SUB):
                rh = pl.multiple_of(t * (TM // 2) + sb * (SUB // 2), 64)
                k = _dot(xn_all[sb * SUB:(sb + 1) * SUB, :], wq[sel, :, D:2 * D])
                if sb == 0:
                    k = k + _tie(qp)
                kk = jnp.where(is_a, _phi(k), k)
                z_acc[...] += jnp.sum(kk.reshape(SUB // 8, 8, D), axis=0)
                kb = _pack(kk)
                for g in range(G):
                    k_s[g, pl.ds(rh, SUB // 2), :] = kb[:, g * 128:(g + 1) * 128]
            return carry

        @pl.when(l > 0)
        def _():
            z_acc[...] = jnp.zeros_like(z_acc)
        lax.fori_loop(jnp.where(l == 0, 1, 0), NTM, body, 0)

    def startup():
        for cp in x0_copies:
            cp.start()
        for cp in wa_copies(0):
            cp.start()
        zero_s[...] = jnp.zeros_like(zero_s)
        xn_b[0:PRE // 2, :] = jnp.zeros((PRE // 2, D), U32)
        for cp in x0_copies[:8]:
            cp.wait()
        xn_0[0:128, :] = _pack(_ln(xin[0:256, :].astype(F32)))
        for cp in x0_copies[8:]:
            cp.wait()
        xn_0[128:256, :] = _pack(_ln(xin[256:512, :].astype(F32)))
        for cp in wa_copies(1):
            cp.start()
        for cp in wa_copies(0):
            cp.wait()

        def body(j, carry):
            xn = _unpack(xn_0[...])
            ct = pl.multiple_of(t_col(j), 256)
            ck = pl.multiple_of(j * 128, 128)
            rc = pl.multiple_of(j * XC, XC)
            xf = xin[pl.ds(rc, XC), :].astype(F32)
            x[pl.ds(rc, XC), :] = xf
            u = pltpu.bitcast(xf, U32)
            u = u[:, 0:512] | u[:, 512:1024]
            u = jnp.concatenate([u[:, 0:256], u[:, 256:512]], axis=0) & jnp.uint32(0x80000000)
            y = (_dot(xn, wq[0, :, pl.ds(ct, 256)]) + pltpu.bitcast(u, F32)).T
            y = jnp.where(j >= 4, _phi(y), y)
            tr = pl.multiple_of((j & 3) * 128, 128)
            t_s[1 - (j >> 2), pl.ds(tr, 128), 0:TM] = _pack(y)
            kk = _phi(_dot(xn, wq[0, :, pl.ds(D + ck, 128)]))
            z_acc[:, pl.ds(ck, 128)] = jnp.sum(kk.reshape(TM // 8, 8, 128), axis=0)
            k_s[j, 0:TM // 2, :] = _pack(kk)
            for c in range(0, PRE, LNC):
                xn1, _ = _ln_chunk(xf[c:c + LNC, :])
                rows = slice(c // 2, (c + LNC) // 2)
                xn_b[rows, :] = jnp.where(j <= TM // XC, _pack(xn1), xn_b[rows, :])

            @pl.when(j + 2 < G)
            def _():
                x_copy(j + 2).start()
                for cp in wa_copies(j + 2):
                    cp.start()

            @pl.when(j == G - 2)
            def _():
                for cp in w_copies:
                    cp.start()

            @pl.when(j + 1 < G)
            def _():
                for cp in wa_copies(j + 1):
                    cp.wait()

                @pl.when(j > 0)
                def _():
                    x_copy(j + 1).wait()
            return carry
        lax.fori_loop(0, G, body, 0)

    def a_mix():
        row = lax.broadcasted_iota(jnp.int32, (128, 128), 0) // DH
        col = lax.broadcasted_iota(jnp.int32, (128, 128), 1) // DH
        same = row == col
        zrow = lax.broadcasted_iota(jnp.int32, (16, 128), 0)
        zcol = lax.broadcasted_iota(jnp.int32, (16, 128), 1) // DH
        zsel = zrow == zcol
        z = jnp.sum(z_acc[...], axis=0, keepdims=True)

        def fold(g, kvg):
            m_s[g * 64:(g + 1) * 64, :] = _pack(_dot(kvg, wo[0, g * 128:(g + 1) * 128, 0:D]))

        def group(g):
            zg = jnp.broadcast_to(z[:, g * 128:(g + 1) * 128], (16, 128))
            zl = jnp.where(zsel, zg, 0.0).astype(BF)
            kvt = None
            for t in range(NTM):
                part = _dot(_unpack(t_s[1, g * 64:(g + 1) * 64, t * TM:(t + 1) * TM]),
                            _unpack(k_s[g, t * TM // 2:(t + 1) * TM // 2, :]))
                kvt = part if kvt is None else kvt + part
                pqt = _unpack(t_s[0, g * 64:(g + 1) * 64, t * TM:(t + 1) * TM])
                r = _recip(_dot(zl, pqt)[0:8, :] + 1e-6)
                pf = pqt.astype(F32)
                ot = jnp.concatenate(
                    [pf[j * DH:(j + 1) * DH, :] * r[j:j + 1, :] for j in range(HPG)], axis=0)
                o_s[g, t * TM // 2:(t + 1) * TM // 2, :] = _pack(ot.T)
            return jnp.where(same, kvt, 0.0).T.astype(BF)

        kvs = []
        for g in range(G):
            kvs.append(group(g))
            if g >= 2:
                fold(g - 2, kvs[g - 2])
        fold(G - 2, kvs[G - 2])
        fold(G - 1, kvs[G - 1])

    def a_out():
        def body(t, carry):
            for sb in range(TM // SUB):
                r0 = pl.multiple_of(t * TM + sb * SUB, SUB)
                rh = pl.multiple_of(t * (TM // 2) + sb * (SUB // 2), SUB // 2)
                o = jnp.concatenate([_unpack(o_s[g, pl.ds(rh, SUB // 2), :]) for g in range(G)], axis=1)
                xnew = x[pl.ds(r0, SUB), :] + _dot(o, _unpack(m_s[...]))
                x[pl.ds(r0, SUB), :] = xnew
                if sb == 0:
                    for c in range(0, PRE, LNC):
                        xn, _ = _ln_chunk(xnew[c:c + LNC, :])
                        rows = slice(c // 2, (c + LNC) // 2)
                        xn_b[rows, :] = jnp.where(t == 0, _pack(xn), xn_b[rows, :])
            return carry
        lax.fori_loop(0, NTM, body, 0)

    def decode(b):
        return b & (G - 1), b >> 3

    def get_qm(b, hh):
        g, qi = decode(b)
        qoff = pl.multiple_of(qi * TQ, TQ)
        roff = pl.multiple_of(g * 64 + hh * 16, 16)
        parts = []
        if hh > 0:
            parts.append(jnp.zeros((hh * 16, TQ), U32))
        parts.append(t_s[0, pl.ds(roff, 16), pl.ds(qoff, TQ)])
        if hh < HPG - 1:
            parts.append(jnp.zeros(((HPG - 1 - hh) * 16, TQ), U32))
        return _unpack(jnp.concatenate(parts, axis=0))

    def qk_chunk(g, qm, c, hh, m8):
        kc = _unpack(k_s[g, c * TK // 2:(c + 1) * TK // 2, :])
        s = _dot(kc, qm)
        s_buf[hh, c * TK:(c + 1) * TK, :] = s
        mc = jnp.max(s.reshape(TK // 8, 8, TQ), axis=0)
        return mc if m8 is None else jnp.maximum(m8, mc)

    def out_proj(b, o):
        g, qi = decode(b)
        r0 = pl.multiple_of(qi * TQ, TQ)
        w0 = pl.multiple_of(g * 128, 128)
        xnew = x[pl.ds(r0, TQ), :] + _dot(o, wo[1, pl.ds(w0, 128), 0:D])
        x[pl.ds(r0, TQ), :] = xnew
        xin[pl.ds(r0, TQ), :] = xnew.astype(BF)

    def lsum(p, l8):
        for r in range(TK // 16 - 1, -1, -1):
            pr = p[r * 16:r * 16 + 8, :] + p[r * 16 + 8:r * 16 + 16, :]
            l8 = pr if l8 is None else l8 + pr
        return l8

    def attn_block(b):
        gc, _ = decode(b)
        gn = (b + 1) & (G - 1)
        o_prev = _unpack(op_s[...])
        outs = []
        ms = [m_buf[hh] for hh in range(HPG)]
        for hh in range(HPG):
            qm = get_qm(b + 1, hh)
            voff = pl.multiple_of(gc * 64 + hh * 16, 16)
            l8 = None
            o = zero_s[...]
            m8 = None
            for c in range(NK):
                p = jnp.exp2(s_buf[hh, c * TK:(c + 1) * TK, :] - ms[hh])
                l8 = lsum(p, l8)
                m8 = qk_chunk(gn, qm, c, hh, m8)
                vc = _unpack(t_s[1, pl.ds(voff, 16), c * TK:(c + 1) * TK])
                o = o + _dot(vc, p.astype(BF))
            m_buf[hh] = jnp.max(m8, axis=0, keepdims=True)
            l = jnp.sum(l8, axis=0, keepdims=True)
            outs.append(o * _recip(l))
        out_proj(jnp.maximum(b - 1, 0), o_prev)
        ot = jnp.concatenate(outs, axis=0)
        op_s[...] = _pack(ot.T)

    def attn_last(is_last_layer):
        rbase = (NQ - 1) * TQ

        def proj_piece(o, g, r, cc, final):
            r0 = rbase + r
            cols = slice(cc * 256, (cc + 1) * 256)
            xnew = x[r0:r0 + 128, cols] + _dot(o, wo[1, g * 128:(g + 1) * 128, cols])
            x[r0:r0 + 128, cols] = xnew
            if final:
                xin[r0:r0 + 128, cols] = xnew.astype(BF)
                if cc == 3:
                    @pl.when(is_last_layer)
                    def _():
                        out_copy_last(r // 128).start()

        o_prev = _unpack(op_s[...])
        queue = [(o_prev[r:r + 128, :], G - 2, r, cc, False) for r in range(0, TQ, 128) for cc in range(4)]
        work = 0
        for q0, q1, ek in ((0, 256, 256), (256, 384, 512), (384, 512, 512)):
            cols = slice(q0, q1)
            outs = []
            for hh in range(HPG):
                m = m_buf[hh, :, cols]
                voff = (G - 1) * 64 + hh * 16
                l8 = None
                o = zero_s[:, 0:q1 - q0]
                for c in range(S // ek):
                    p = jnp.exp2(s_buf[hh, c * ek:(c + 1) * ek, cols] - m)
                    for u in range(ek // TK):
                        l8 = lsum(p[u * TK:(u + 1) * TK, :], l8)
                    vc = _unpack(t_s[1, voff:voff + 16, c * ek:(c + 1) * ek])
                    o = o + _dot(vc, p.astype(BF))
                    work += ek * (q1 - q0) // 1024
                    while queue and work >= 128:
                        work -= 128
                        proj_piece(*queue.pop(0))
                    if not queue:
                        work = 0
                l = jnp.sum(l8, axis=0, keepdims=True)
                outs.append(o * _recip(l))
            oj = jnp.concatenate(outs, axis=0).T.astype(BF)
            if not queue:
                work = -192
            queue += [(oj[r:r + 128, :], G - 1, q0 + r, cc, True) for r in range(0, q1 - q0, 128) for cc in range(4)]
        while queue:
            proj_piece(*queue.pop(0))

    def attention(is_last_layer):
        op_s[...] = jnp.zeros_like(op_s)
        for hh in range(HPG):
            qm = get_qm(0, hh)
            m8 = None
            for c in range(NK):
                m8 = qk_chunk(0, qm, c, hh, m8)
            m_buf[hh] = jnp.max(m8, axis=0, keepdims=True)

        def body(b, carry):
            @pl.when(jnp.logical_and(is_last_layer, jnp.logical_and((b & (G - 1)) == 1, b > G)))
            def _():
                out_copy((b >> 3) - 1).start()
            attn_block(b)
            return carry
        lax.fori_loop(0, NBLK - 1, body, 0)
        ln_rows(0, 0, PRE)
        attn_last(is_last_layer)

    startup()

    def layer(l, carry):
        sel = l & 1
        q_phase(l)

        @pl.when(l == 0)
        def _():
            for cp in w_copies:
                cp.wait()

        @pl.when(sel == 0)
        def _():
            a_mix()
            a_out()

        @pl.when(sel == 1)
        def _():
            attention(l == 3)
        return carry

    lax.fori_loop(0, 4, layer, 0)
    for t in range(NTM - 1):
        out_copy(t).wait()
    for j in range(TM // 128):
        out_copy_last(j).wait()


@jax.jit
def pallas_interleave_layers__linear_attn_block__mha_block__prompt_kernel(A_x, A_wqkv, A_wo, B_x, B_wqkv, B_wo):
    del B_x
    scratch = [
        pltpu.VMEM((S, D), BF),
        pltpu.VMEM((S, D), F32),
        pltpu.VMEM((TM // 2, D), U32),
        pltpu.VMEM((TM // 2, D), U32),
        pltpu.VMEM((2, D, 3 * D + WPAD), BF),
        pltpu.VMEM((2, D, D + WPAD), BF),
        pltpu.VMEM((2, D // 2, S), U32),
        pltpu.VMEM((G, S // 2, 128), U32),
        pltpu.VMEM((G, S // 2, 128), U32),
        pltpu.VMEM((TQ // 2, 128), U32),
        pltpu.VMEM((8, D), F32),
        pltpu.VMEM((D // 2, D), U32),
        pltpu.VMEM((DH, TQ), F32),
        pltpu.VMEM((HPG, S, TQ), F32),
        pltpu.VMEM((HPG, 1, TQ), F32),
        pltpu.SemaphoreType.DMA((2,)),
        pltpu.SemaphoreType.DMA((2,)),
        pltpu.SemaphoreType.DMA((1,)),
        pltpu.SemaphoreType.DMA((1,)),
    ]
    out = pl.pallas_call(
        _kernel,
        out_shape=jax.ShapeDtypeStruct((S, D), BF),
        in_specs=[pl.BlockSpec(memory_space=pl.ANY)] * 5,
        out_specs=pl.BlockSpec(memory_space=pl.ANY),
        scratch_shapes=scratch,
        compiler_params=pltpu.CompilerParams(
            vmem_limit_bytes=120 * 1024 * 1024,
            disable_bounds_checks=True,
        ),
    )(A_x.reshape(S, D), A_wqkv, A_wo, B_wqkv, B_wo)
    return out.reshape(1, S, D)
```
